```python
import jax
import jax.numpy as jnp

def _softmax(x, axis=-1):
    return jax.nn.softmax(x, axis=axis)

def _gelu(x):
    return jax.nn.gelu(x, approximate=True)

def _silu(x):
    return jax.nn.silu(x)

def _sigmoid(x):
    return jax.nn.sigmoid(x)

def _layernorm(x, axis=-1, eps=1e-05):
    m = jnp.mean(x, axis=axis, keepdims=True)
    v = jnp.var(x, axis=axis, keepdims=True)
    return (x - m) / jnp.sqrt(v + eps)

def _scatter_add(tgt, idx, src, axis=0):
    return tgt.at[idx].add(src)

def _segment_sum(src, seg, n):
    return jax.ops.segment_sum(src, seg, n)

class _Rng:

    def __init__(self, key):
        self._k = key

    def _next(self):
        self._k, sub = jax.random.split(self._k)
        return sub

    def normal(self, shape):
        return jax.random.normal(self._next(), shape, dtype=jnp.bfloat16)

    def randint(self, lo, hi, shape):
        return jax.random.randint(self._next(), shape, lo, hi, dtype=jnp.int32)

    def uniform(self, shape, lo=0.0, hi=1.0):
        return jax.random.uniform(self._next(), shape, jnp.bfloat16, lo, hi)

    def permutation(self, n):
        return jax.random.permutation(self._next(), n)
kernel_name = 'adaLN_cond__ssm_conv_h3__dense_activation_gelu__prompt'

def setup_inputs():
    _rng = _Rng(jax.random.key(int.from_bytes(__import__("os").urandom(4), "little")))
    _w = lambda a: (lambda t: t.astype(jnp.bfloat16) if jnp.issubdtype(t.dtype, jnp.floating) else t)(jnp.asarray(a))

    def _A_setup():
        B, S, D = (1, 2048, 640)
        ks = 4
        return {'q': _w((lambda *s: _rng.normal(s) * 0.05)(B, S, D)), 'k': _w((lambda *s: _rng.normal(s) * 0.05)(B, S, D)), 'v': _w((lambda *s: _rng.normal(s) * 0.05)(B, S, D)), 'shift_k': _w((lambda *s: _rng.normal(s) * 0.05)(D, ks) * 0.5), 'ssm_k': _w((lambda *s: _rng.normal(s) * 0.05)(D, S) * (1.0 / S ** 0.5)), 'ssm_D': _w((lambda *s: _rng.normal(s) * 0.05)(D))}
    _A_in = _A_setup()

    def _B_setup():
        B, S, D, F = (1, 2048, 640, 1728)
        return {'x': _w((lambda *s: _rng.normal(s) * 0.05)(B, S, D)), 'w1': _w((lambda *s: _rng.normal(s) * 0.05)(D, F) * D ** (-0.5)), 'b1': _w((lambda *s: _rng.normal(s) * 0.05)(F) * 0.01), 'w2': _w((lambda *s: _rng.normal(s) * 0.05)(F, D) * F ** (-0.5)), 'b2': _w((lambda *s: _rng.normal(s) * 0.05)(D) * 0.01)}
    _B_in = _B_setup()
    return {'A_q': _A_in['q'], 'A_k': _A_in['k'], 'A_v': _A_in['v'], 'A_shift_k': _A_in['shift_k'], 'A_ssm_k': _A_in['ssm_k'], 'A_ssm_D': _A_in['ssm_D'], 'B_x': _B_in['x'], 'B_w1': _B_in['w1'], 'B_b1': _B_in['b1'], 'B_w2': _B_in['w2'], 'B_b2': _B_in['b2'], 'c': _w((lambda *s: _rng.normal(s) * 0.05)(1, 640)), 'w_mod': _w((lambda *s: _rng.normal(s) * 0.05)(640, 6 * 640) * 640 ** (-0.5))}

def reference(A_q, A_k, A_v, A_shift_k, A_ssm_k, A_ssm_D, B_x, B_w1, B_b1, B_w2, B_b2, c, w_mod):

    def _A_ref(q, k, v, shift_k, ssm_k, ssm_D):
        B, S, D = q.shape
        ks = shift_k.shape[-1]
        k_pad = jnp.pad(k, ((0, 0), (ks - 1, 0), (0, 0)))
        k_shift = jnp.zeros_like(k)
        for t in range(ks):
            k_shift = k_shift + k_pad[:, t:t + S, :] * shift_k[:, ks - 1 - t][None, None, :]
        kv = k_shift * v
        L = 2 * S
        kv_pad = jnp.pad(kv, ((0, 0), (0, S), (0, 0)))
        kf_pad = jnp.pad(ssm_k, ((0, 0), (0, S)))
        kv_f = (lambda x, axes=(-2, -1): jnp.fft.rfft2(x.astype(jnp.float32), axes=axes))(kv_pad[:, None, :, :], axes=(1, 2))
        kf_f = (lambda x, axes=(-2, -1): jnp.fft.rfft2(x.astype(jnp.float32), axes=axes))(kf_pad[:, None, :], axes=(1, 2))
        kf_f = (lambda x, *d: x.transpose(*d))(kf_f, 1, 2, 0)
        y_f = kv_f * kf_f[None, :, :, :]
        y = (lambda x, s, axes=(-2, -1): jnp.fft.irfft2(x, s=s, axes=axes).astype(jnp.bfloat16))(y_f, (1, L), axes=(1, 2))[:, 0, :S, :]
        y = y + kv * ssm_D[None, None, :]
        return q * y

    def _B_ref(x, w1, b1, w2, b2):
        h = jnp.einsum('bsd,df->bsf', x, w1) + b1
        h = _gelu(h)
        return jnp.einsum('bsf,fd->bsd', h, w2) + b2
    x = A_q
    mod = (_silu(c) @ w_mod).reshape(c.shape[0], 6, 1, -1)
    sa, ca, ga, sb, cb, gb = (mod[:, 0].copy(), mod[:, 1].copy(), mod[:, 2].copy(), mod[:, 3].copy(), mod[:, 4].copy(), mod[:, 5].copy())
    h = _layernorm(x, axis=-1) * (1 + ca) + sa
    x = x + ga * _A_ref(h, A_k, A_v, A_shift_k, A_ssm_k, A_ssm_D)
    h = _layernorm(x, axis=-1) * (1 + cb) + sb
    x = x + gb * _B_ref(h, B_w1, B_b1, B_w2, B_b2)
    return x
```

```python
import numpy as np
import jax
import jax.numpy as jnp
from jax import lax
import jax.experimental.pallas as pl
import jax.experimental.pallas.tpu as pltpu

S, D, F = 2048, 640, 1728
C = 128
NC = S // C
NT = D // 128
HALO = 16
TM = 256
f32, bf16 = jnp.float32, jnp.bfloat16


def _dft_consts():
    f = np.arange(C, dtype=np.float64)[:, None] + 0.5
    t = np.arange(C, dtype=np.float64)[None, :]
    th = 2.0 * np.pi * f * t / (2 * C)
    fwd = np.concatenate([np.cos(th), -np.sin(th)], axis=0)
    inv = np.concatenate([np.cos(th).T, -np.sin(th).T], axis=1) / C
    return fwd.astype(np.float32), inv.astype(np.float32)


def _ln(x):
    m = jnp.mean(x, axis=-1, keepdims=True)
    xc = x - m
    v = jnp.mean(xc * xc, axis=-1, keepdims=True)
    return xc * lax.rsqrt(v + 1e-5)


def _kernel(q_h, k_h, v_h, shk_ref, ssm_h, ssd_ref, w1_h, b1_ref, w2_h, b2_ref, c_ref, wm_h,
            fwd_ref, inv_ref, o_h,
            qb, kb, vb, sb, w1b, w2b, wmb, kvs, ys, xs, ks, kprev, zs, ob, sem_in, sem_w, sem_o):
    def slab(c):
        cols = pl.ds(c * 128, 128)
        return (pltpu.make_async_copy(k_h.at[0, :, cols], kb.at[c, pl.ds(HALO, S)], sem_in.at[0, c]),
                pltpu.make_async_copy(v_h.at[0, :, cols], vb.at[c], sem_in.at[1, c]),
                pltpu.make_async_copy(ssm_h.at[cols, :], sb.at[c], sem_in.at[2, c]))
    for c in range(NT):
        for cp in slab(c):
            cp.start()
    cp_wm = pltpu.make_async_copy(wm_h, wmb, sem_w.at[0])
    cp_q = pltpu.make_async_copy(q_h.at[0], qb, sem_w.at[1])
    cp_w1 = pltpu.make_async_copy(w1_h, w1b, sem_w.at[2])
    cp_w2 = pltpu.make_async_copy(w2_h, w2b, sem_w.at[3])
    for cp in (cp_wm, cp_q, cp_w1, cp_w2):
        cp.start()

    for c in range(NT):
        kb[c, pl.ds(0, HALO), :] = jnp.zeros((HALO, 128), bf16)

    sel = (lax.broadcasted_iota(jnp.int32, (8, 4), 0) == lax.broadcasted_iota(jnp.int32, (8, 4), 1)).astype(bf16)
    taps = lax.dot_general(sel, shk_ref[...], (((1,), (1,)), ((), ())), preferred_element_type=f32)
    ssd = ssd_ref[...].astype(f32)
    sigma = (1 - 2 * (lax.broadcasted_iota(jnp.int32, (C, 128), 0) & 1)).astype(f32)

    def aligned(i, n):
        return pl.ds(pl.multiple_of(i * n, n), n)

    def stage_a(c, j):
        slot = c % 2
        lo, hi = c * 128, (c + 1) * 128
        w = kb[c, pl.ds(pl.multiple_of(j * C, C), C + HALO), :].astype(f32)
        ksh = w[HALO:] * taps[0:1, lo:hi]
        for s in range(1, 4):
            ksh = ksh + w[HALO - s:HALO - s + C] * taps[s:s + 1, lo:hi]
        kv = ksh * vb[c, aligned(j, C), :].astype(f32)
        kvs[c, aligned(j, C), :] = kv
        fw = fwd_ref[...]
        xh = jnp.dot(fw, kv.astype(bf16), preferred_element_type=f32)
        a, b = xh[:C], xh[C:]
        xs[slot, j, 0] = a
        xs[slot, j, 1] = b
        xs[slot, j, 2] = a + b
        kh = lax.dot_general(fw, sb[c, :, aligned(j, C)], (((1,), (1,)), ((), ())),
                             preferred_element_type=f32)
        kc, kd = kh[:C], kh[C:]
        cc = kc - sigma * kprev[1]
        dd = kd + sigma * kprev[0]
        kprev[0] = kc
        kprev[1] = kd
        ks[slot, j, 0] = cc
        ks[slot, j, 1] = dd - cc
        ks[slot, j, 2] = cc + dd

    def stage_b(c, ft):
        slot = c % 2
        rows = aligned(ft, 8)
        IB = 4
        for i0 in range(0, NC, IB):
            acc = [[None] * 3 for _ in range(IB)]
            kreg = {}
            for j in range(i0 + IB):
                xa, xb, xab = (xs[slot, j, 2, rows, :], xs[slot, j, 0, rows, :], xs[slot, j, 1, rows, :])
                for ii in range(IB):
                    m = i0 + ii - j
                    if m < 0:
                        continue
                    if m not in kreg:
                        kreg[m] = tuple(ks[slot, m, p, rows, :] for p in range(3))
                    for p, xv in enumerate((xa, xb, xab)):
                        t = kreg[m][p] * xv
                        acc[ii][p] = t if acc[ii][p] is None else acc[ii][p] + t
                kreg.pop(i0 - j, None)
            for ii in range(IB):
                zs[slot, i0 + ii, rows, :] = acc[ii][0] - acc[ii][2]
                zs[slot, i0 + ii, pl.ds(pl.multiple_of(C + ft * 8, 8), 8), :] = acc[ii][0] + acc[ii][1]

    def stage_c(c, i):
        slot = c % 2
        y = jnp.dot(inv_ref[...], zs[slot, i].astype(bf16), preferred_element_type=f32)
        ys[c, aligned(i, C), :] = y + kvs[c, aligned(i, C), :] * ssd[:, c * 128:(c + 1) * 128]

    for c in range(-1, NT + 1):
        if 0 <= c + 1 < NT:
            for cp in slab(c + 1):
                cp.wait()
            kprev[...] = jnp.zeros_like(kprev)

        def body(t, _, c=c):
            if 0 <= c + 1 < NT:
                stage_a(c + 1, t)
            if 0 <= c < NT:
                stage_b(c, t)
            if 0 <= c - 1 < NT:
                stage_c(c - 1, t)
            return 0
        lax.fori_loop(0, NC, body, 0)

    cp_wm.wait()
    cv = c_ref[...].astype(f32)
    sc = (cv * jax.nn.sigmoid(cv)).astype(bf16)
    mod = jnp.dot(jnp.broadcast_to(sc, (8, D)), wmb[...], preferred_element_type=f32)[0:1]
    sa, ca, ga, sbb, cb, gb = (mod[:, n * D:(n + 1) * D] for n in range(6))
    b1 = b1_ref[...].astype(f32)
    b2 = b2_ref[...].astype(f32)
    cp_q.wait()
    cp_w1.wait()
    cp_w2.wait()

    def out_copy(r, slot):
        return pltpu.make_async_copy(ob.at[slot], o_h.at[0, aligned(r, TM), :], sem_o.at[slot])

    def ffn(r, _):
        rows = aligned(r, TM)
        slot = r % 2
        x0 = qb[rows, :].astype(f32)
        y = jnp.concatenate([ys[c, rows, :] for c in range(NT)], axis=1)
        x1 = x0 + ga * ((_ln(x0) * (1.0 + ca) + sa) * y)
        h2 = (_ln(x1) * (1.0 + cb) + sbb).astype(bf16)
        h = jnp.dot(h2, w1b[...], preferred_element_type=f32) + b1
        g = jax.nn.gelu(h, approximate=True).astype(bf16)
        o = jnp.dot(g, w2b[...], preferred_element_type=f32) + b2

        @pl.when(r >= 2)
        def _():
            out_copy(r - 2, slot).wait()
        ob[slot] = (x1 + gb * o).astype(bf16)
        out_copy(r, slot).start()
        return 0
    lax.fori_loop(0, S // TM, ffn, 0)
    out_copy(S // TM - 2, 0).wait()
    out_copy(S // TM - 1, 1).wait()


@jax.jit
def pallas_adaLN_cond__ssm_conv_h3__dense_activation_gelu__prompt_kernel(
    A_q, A_k, A_v, A_shift_k, A_ssm_k, A_ssm_D, B_x, B_w1, B_b1, B_w2, B_b2, c, w_mod,
):
    del B_x
    fwd, inv = _dft_consts()
    hbm = pl.BlockSpec(memory_space=pl.ANY)
    vm = pl.BlockSpec(memory_space=pltpu.VMEM)
    return pl.pallas_call(
        _kernel,
        in_specs=[hbm, hbm, hbm, vm, hbm, vm, hbm, vm, hbm, vm, vm, hbm, vm, vm],
        out_specs=hbm,
        out_shape=jax.ShapeDtypeStruct((1, S, D), bf16),
        scratch_shapes=[
            pltpu.VMEM((S, D), bf16),
            pltpu.VMEM((NT, S + HALO, 128), bf16),
            pltpu.VMEM((NT, S, 128), bf16),
            pltpu.VMEM((NT, 128, S), bf16),
            pltpu.VMEM((D, F), bf16),
            pltpu.VMEM((F, D), bf16),
            pltpu.VMEM((D, 6 * D), bf16),
            pltpu.VMEM((NT, S, 128), f32),
            pltpu.VMEM((NT, S, 128), f32),
            pltpu.VMEM((2, NC, 3, C, 128), f32),
            pltpu.VMEM((2, NC, 3, C, 128), f32),
            pltpu.VMEM((2, C, 128), f32),
            pltpu.VMEM((2, NC, 2 * C, 128), f32),
            pltpu.VMEM((2, TM, D), bf16),
            pltpu.SemaphoreType.DMA((3, NT)),
            pltpu.SemaphoreType.DMA((4,)),
            pltpu.SemaphoreType.DMA((2,)),
        ],
        compiler_params=pltpu.CompilerParams(vmem_limit_bytes=100 * 1024 * 1024),
    )(A_q, A_k, A_v, A_shift_k, A_ssm_k, A_ssm_D.reshape(1, D), B_w1, B_b1.reshape(1, F),
      B_w2, B_b2.reshape(1, D), c, w_mod, jnp.asarray(fwd, bf16), jnp.asarray(inv, bf16))
```

```python
import numpy as np
import jax
import jax.numpy as jnp
from jax import lax
import jax.experimental.pallas as pl
import jax.experimental.pallas.tpu as pltpu

S, D, F = 2048, 640, 1728
C = 128
NC = S // C
NT = D // 128
HALO = 16
TM = 256
f32, bf16 = jnp.float32, jnp.bfloat16


def _dft_consts():
    f = np.arange(C, dtype=np.float64)[:, None] + 0.5
    t = np.arange(C, dtype=np.float64)[None, :]
    th = 2.0 * np.pi * f * t / (2 * C)
    fwd = np.concatenate([np.cos(th), -np.sin(th)], axis=0)
    inv = np.concatenate([np.cos(th).T, -np.sin(th).T], axis=1) / C
    return fwd.astype(np.float32), inv.astype(np.float32)


def _ln(x):
    m = jnp.mean(x, axis=-1, keepdims=True)
    xc = x - m
    v = jnp.mean(xc * xc, axis=-1, keepdims=True)
    return xc * lax.rsqrt(v + 1e-5)


def _kernel(q_h, k_h, v_h, shk_ref, ssm_h, ssd_ref, w1_h, b1_ref, w2_h, b2_ref, c_ref, wm_h,
            fwd_ref, inv_ref, o_h,
            qb, kb, vb, sb, w1b, w2b, wmb, kprev, ob, sem_in, sem_w, sem_o, *rest):
    kvs, ys = rest[:NT], rest[NT:2 * NT]
    xs, ks, zs = (rest[2 * NT + 2 * n:2 * NT + 2 * n + 2] for n in range(3))
    def slab(c):
        cols = pl.ds(c * 128, 128)
        return (pltpu.make_async_copy(k_h.at[0, :, cols], kb.at[c, pl.ds(HALO, S)], sem_in.at[0, c]),
                pltpu.make_async_copy(v_h.at[0, :, cols], vb.at[c], sem_in.at[1, c]),
                pltpu.make_async_copy(ssm_h.at[cols, :], sb.at[c], sem_in.at[2, c]))
    for c in range(NT):
        for cp in slab(c):
            cp.start()
    cp_wm = pltpu.make_async_copy(wm_h, wmb, sem_w.at[0])
    cp_q = pltpu.make_async_copy(q_h.at[0], qb, sem_w.at[1])
    cp_w1 = pltpu.make_async_copy(w1_h, w1b, sem_w.at[2])
    cp_w2 = pltpu.make_async_copy(w2_h, w2b, sem_w.at[3])
    for cp in (cp_wm, cp_q, cp_w1, cp_w2):
        cp.start()

    for c in range(NT):
        kb[c, pl.ds(0, HALO), :] = jnp.zeros((HALO, 128), bf16)


    taps = shk_ref[...].astype(f32)
    ssd = ssd_ref[...].reshape(1, D).astype(f32)
    sigma = (1 - 2 * (lax.broadcasted_iota(jnp.int32, (C, 128), 0) & 1)).astype(f32)

    def aligned(i, n):
        return pl.ds(pl.multiple_of(i * n, n), n)

    def stage_a(c, j):
        slot = c % 2
        lo, hi = c * 128, (c + 1) * 128
        w = kb[c, pl.ds(pl.multiple_of(j * C, C), C + HALO), :].astype(f32)
        ksh = w[HALO:] * taps[0:1, lo:hi]
        for s in range(1, 4):
            ksh = ksh + w[HALO - s:HALO - s + C] * taps[s:s + 1, lo:hi]
        kv = ksh * vb[c, aligned(j, C), :].astype(f32)
        kvs[c][aligned(j, C), :] = kv
        fw = fwd_ref[...]
        xh = jnp.dot(fw, kv.astype(bf16), preferred_element_type=f32)
        a, b = xh[:C], xh[C:]
        xs[slot][j, 0] = a
        xs[slot][j, 1] = b
        xs[slot][j, 2] = a + b
        kh = lax.dot_general(fw, sb[c, :, aligned(j, C)], (((1,), (1,)), ((), ())),
                             preferred_element_type=f32)
        kc, kd = kh[:C], kh[C:]
        cc = kc - sigma * kprev[1]
        dd = kd + sigma * kprev[0]
        kprev[0] = kc
        kprev[1] = kd
        ks[slot][j, 0] = cc
        ks[slot][j, 1] = dd - cc
        ks[slot][j, 2] = cc + dd

    def stage_b(c, ft):
        slot = c % 2
        rows = aligned(ft, 8)
        IB = 4
        for i0 in range(0, NC, IB):
            acc = [[None] * 3 for _ in range(IB)]
            kreg = {}
            for j in range(i0 + IB):
                xa, xb, xab = (xs[slot][j, 2, rows, :], xs[slot][j, 0, rows, :], xs[slot][j, 1, rows, :])
                for ii in range(IB):
                    m = i0 + ii - j
                    if m < 0:
                        continue
                    if m not in kreg:
                        kreg[m] = tuple(ks[slot][m, p, rows, :] for p in range(3))
                    for p, xv in enumerate((xa, xb, xab)):
                        t = kreg[m][p] * xv
                        acc[ii][p] = t if acc[ii][p] is None else acc[ii][p] + t
                kreg.pop(i0 - j, None)
            for ii in range(IB):
                zs[slot][i0 + ii, rows, :] = acc[ii][0] - acc[ii][2]
                zs[slot][i0 + ii, pl.ds(pl.multiple_of(C + ft * 8, 8), 8), :] = acc[ii][0] + acc[ii][1]

    def stage_c(c, i):
        slot = c % 2
        y = jnp.dot(inv_ref[...], zs[slot][i].astype(bf16), preferred_element_type=f32)
        ys[c][aligned(i, C), :] = y + kvs[c][aligned(i, C), :] * ssd[:, c * 128:(c + 1) * 128]

    for c in range(-1, NT + 1):
        if 0 <= c + 1 < NT:
            for cp in slab(c + 1):
                cp.wait()
            kprev[...] = jnp.zeros_like(kprev)

        def body(t, _, c=c):
            if 0 <= c + 1 < NT:
                stage_a(c + 1, t)
            if 0 <= c < NT:
                stage_b(c, t)
            if 0 <= c - 1 < NT:
                stage_c(c - 1, t)
            return 0
        with jax.named_scope('conv%d' % (c + 1)):
            lax.fori_loop(0, NC, body, 0)

    cp_wm.wait()
    cv = c_ref[...].astype(f32)
    sc = (cv * jax.nn.sigmoid(cv)).astype(bf16)
    mod = jnp.dot(jnp.broadcast_to(sc, (8, D)), wmb[...], preferred_element_type=f32)[0:1]
    sa, ca, ga, sbb, cb, gb = (mod[:, n * D:(n + 1) * D] for n in range(6))
    b1 = b1_ref[...].reshape(1, F).astype(f32)
    b2 = b2_ref[...].reshape(1, D).astype(f32)
    cp_q.wait()
    cp_w1.wait()
    cp_w2.wait()

    def out_copy(r, slot):
        return pltpu.make_async_copy(ob.at[slot], o_h.at[0, aligned(r, TM), :], sem_o.at[slot])

    def ffn(r, _):
        rows = aligned(r, TM)
        slot = r % 2
        x0 = qb[rows, :].astype(f32)
        y = jnp.concatenate([ys[c][rows, :] for c in range(NT)], axis=1)
        x1 = x0 + ga * ((_ln(x0) * (1.0 + ca) + sa) * y)
        h2 = (_ln(x1) * (1.0 + cb) + sbb).astype(bf16)
        h = lax.dot_general(h2, w1b[...], (((1,), (1,)), ((), ())), preferred_element_type=f32) + b1
        g = jax.nn.gelu(h, approximate=True).astype(bf16)
        o = jnp.dot(g, w2b[...], preferred_element_type=f32) + b2

        @pl.when(r >= 2)
        def _():
            out_copy(r - 2, slot).wait()
        ob[slot] = (x1 + gb * o).astype(bf16)
        out_copy(r, slot).start()
        return 0
    with jax.named_scope('ffn'):
        lax.fori_loop(0, S // TM, ffn, 0)
    out_copy(S // TM - 2, 0).wait()
    out_copy(S // TM - 1, 1).wait()


@jax.jit
def pallas_adaLN_cond__ssm_conv_h3__dense_activation_gelu__prompt_kernel(
    A_q, A_k, A_v, A_shift_k, A_ssm_k, A_ssm_D, B_x, B_w1, B_b1, B_w2, B_b2, c, w_mod,
):
    del B_x
    fwd, inv = _dft_consts()
    hbm = pl.BlockSpec(memory_space=pltpu.HBM)
    vm = pl.BlockSpec(memory_space=pltpu.VMEM)
    return pl.pallas_call(
        _kernel,
        in_specs=[hbm, hbm, hbm, vm, hbm, vm, hbm, vm, hbm, vm, vm, hbm, vm, vm],
        out_specs=hbm,
        out_shape=jax.ShapeDtypeStruct((1, S, D), bf16),
        scratch_shapes=[
            pltpu.VMEM((S, D), bf16),
            pltpu.VMEM((NT, S + HALO, 128), bf16),
            pltpu.VMEM((NT, S, 128), bf16),
            pltpu.VMEM((NT, 128, S), bf16),
            pltpu.VMEM((F, D), bf16),
            pltpu.VMEM((F, D), bf16),
            pltpu.VMEM((D, 6 * D), bf16),
            pltpu.VMEM((2, C, 128), f32),
            pltpu.VMEM((2, TM, D), bf16),
            pltpu.SemaphoreType.DMA((3, NT)),
            pltpu.SemaphoreType.DMA((4,)),
            pltpu.SemaphoreType.DMA((2,)),
        ] + [pltpu.VMEM((S, 128), f32)] * (2 * NT)
          + [pltpu.VMEM((NC, 3, C, 128), f32)] * 4
          + [pltpu.VMEM((NC, 2 * C, 128), f32)] * 2,
        compiler_params=pltpu.CompilerParams(vmem_limit_bytes=100 * 1024 * 1024),
    )(A_q, A_k, A_v, A_shift_k.T, A_ssm_k, A_ssm_D, B_w1.T, B_b1,
      B_w2, B_b2, c, w_mod, jnp.asarray(fwd, bf16), jnp.asarray(inv, bf16))
```

```python
import numpy as np
import jax
import jax.numpy as jnp
from jax import lax
import jax.experimental.pallas as pl
import jax.experimental.pallas.tpu as pltpu

S, D, F = 2048, 640, 1728
C = 128
NC = S // C
NT = D // 128
HALO = 16
FCUTS = (0,1024,F)
TM = 256
f32, bf16 = jnp.float32, jnp.bfloat16


def _dft_consts():
    f = np.arange(C, dtype=np.float64)[:, None] + 0.5
    t = np.arange(C, dtype=np.float64)[None, :]
    th = 2.0 * np.pi * f * t / (2 * C)
    fwd = np.concatenate([np.cos(th), -np.sin(th)], axis=0)
    inv = np.concatenate([np.cos(th).T, -np.sin(th).T], axis=1) / C
    return fwd.astype(np.float32), inv.astype(np.float32)


def _ln(x):
    m = jnp.mean(x, axis=-1, keepdims=True)
    xc = x - m
    v = jnp.mean(xc * xc, axis=-1, keepdims=True)
    return xc * lax.rsqrt(v + 1e-5)


def _kernel(q_h, k_h, v_h, shk_ref, ssm_h, ssd_ref, w1_h, b1_ref, w2_h, b2_ref, c_ref, wm_h,
            fwd_ref, inv_ref, o_h,
            qb, kb, vb, sb, w1b, w2b, wmb, kprev, ob, x1b, h2b, sem_in, sem_w, sem_o, *rest):
    kvs, ys = rest[:NT], rest[NT:2 * NT]
    xs, ks, zs = (rest[2 * NT + 2 * n:2 * NT + 2 * n + 2] for n in range(3))
    def slab(c):
        cols = pl.ds(c * 128, 128)
        return (pltpu.make_async_copy(k_h.at[0, :, cols], kb.at[c, pl.ds(HALO, S)], sem_in.at[0, c]),
                pltpu.make_async_copy(v_h.at[0, :, cols], vb.at[c], sem_in.at[1, c]),
                pltpu.make_async_copy(ssm_h.at[cols, :], sb.at[c], sem_in.at[2, c]))
    for c in range(NT):
        for cp in slab(c):
            cp.start()
    cp_wm = pltpu.make_async_copy(wm_h, wmb, sem_w.at[0])
    cp_q = pltpu.make_async_copy(q_h.at[0], qb, sem_w.at[1])
    cp_w1 = pltpu.make_async_copy(w1_h, w1b, sem_w.at[2])
    cp_w2 = pltpu.make_async_copy(w2_h, w2b, sem_w.at[3])

    for c in range(NT):
        kb[c, pl.ds(0, HALO), :] = jnp.zeros((HALO, 128), bf16)


    taps = shk_ref[...].astype(f32)
    ssd = ssd_ref[...].reshape(1, D).astype(f32)
    sigma = (1 - 2 * (lax.broadcasted_iota(jnp.int32, (C, 128), 0) & 1)).astype(f32)

    def aligned(i, n):
        return pl.ds(pl.multiple_of(i * n, n), n)

    def stage_a(c, j):
        slot = c % 2
        lo, hi = c * 128, (c + 1) * 128
        w = kb[c, pl.ds(pl.multiple_of(j * C, C), C + HALO), :].astype(f32)
        ksh = w[HALO:] * taps[0:1, lo:hi]
        for s in range(1, 4):
            ksh = ksh + w[HALO - s:HALO - s + C] * taps[s:s + 1, lo:hi]
        kv = ksh * vb[c, aligned(j, C), :].astype(f32)
        kvs[c][aligned(j, C), :] = kv
        fw = fwd_ref[...]
        xh = jnp.dot(fw, kv.astype(bf16), preferred_element_type=f32)
        a, b = xh[:C], xh[C:]
        xs[slot][j, 0] = a
        xs[slot][j, 1] = b
        xs[slot][j, 2] = a + b
        kh = lax.dot_general(fw, sb[c, :, aligned(j, C)], (((1,), (1,)), ((), ())),
                             preferred_element_type=f32)
        kc, kd = kh[:C], kh[C:]
        cc = kc - sigma * kprev[1]
        dd = kd + sigma * kprev[0]
        kprev[0] = kc
        kprev[1] = kd
        ks[slot][j, 0] = cc
        ks[slot][j, 1] = dd - cc
        ks[slot][j, 2] = cc + dd

    def stage_b(c, ft):
        slot = c % 2
        rows = aligned(ft, 8)
        IB = 4
        for i0 in range(0, NC, IB):
            acc = [[None] * 3 for _ in range(IB)]
            kreg = {}
            for j in range(i0 + IB):
                xa, xb, xab = (xs[slot][j, 2, rows, :], xs[slot][j, 0, rows, :], xs[slot][j, 1, rows, :])
                for ii in range(IB):
                    m = i0 + ii - j
                    if m < 0:
                        continue
                    if m not in kreg:
                        kreg[m] = tuple(ks[slot][m, p, rows, :] for p in range(3))
                    for p, xv in enumerate((xa, xb, xab)):
                        t = kreg[m][p] * xv
                        acc[ii][p] = t if acc[ii][p] is None else acc[ii][p] + t
                kreg.pop(i0 - j, None)
            for ii in range(IB):
                zs[slot][i0 + ii, rows, :] = acc[ii][0] - acc[ii][2]
                zs[slot][i0 + ii, pl.ds(pl.multiple_of(C + ft * 8, 8), 8), :] = acc[ii][0] + acc[ii][1]

    def stage_c(c, i):
        slot = c % 2
        y = jnp.dot(inv_ref[...], zs[slot][i].astype(bf16), preferred_element_type=f32)
        ys[c][aligned(i, C), :] = y + kvs[c][aligned(i, C), :] * ssd[:, c * 128:(c + 1) * 128]

    for c in range(-1, NT + 1):
        if 0 <= c + 1 < NT:
            with jax.named_scope('wait%d' % (c + 1)):
                for cp in slab(c + 1):
                    cp.wait()
            for cp in {0: (cp_wm,), 1: (cp_q, cp_w1, cp_w2)}.get(c, ()):
                cp.start()
            kprev[...] = jnp.zeros_like(kprev)

        def body(t, _, c=c):
            if 0 <= c + 1 < NT:
                stage_a(c + 1, t)
            if 0 <= c < NT:
                stage_b(c, t)
            if 0 <= c - 1 < NT:
                stage_c(c - 1, t)
            return 0
        with jax.named_scope('conv%d' % (c + 1)):
            lax.fori_loop(0, NC, body, 0, unroll=16)

    with jax.named_scope('mod'):
        cp_wm.wait()
        cv = c_ref[...].astype(f32)
        sc = (cv * jax.nn.sigmoid(cv)).astype(bf16)
        mod = jnp.dot(jnp.broadcast_to(sc, (8, D)), wmb[...], preferred_element_type=f32)[0:1]
        sa, ca, ga, sbb, cb, gb = (mod[:, n * D:(n + 1) * D] for n in range(6))
        b1 = b1_ref[...].reshape(1, F).astype(f32)
        b2 = b2_ref[...].reshape(1, D).astype(f32)
        cp_q.wait()
        cp_w1.wait()
        cp_w2.wait()

    def out_copy(r, slot):
        return pltpu.make_async_copy(ob.at[slot], o_h.at[0, aligned(r, TM), :], sem_o.at[slot])

    def prep(r, slot):
        rows = aligned(r, TM)
        x0 = qb[rows, :].astype(f32)
        y = jnp.concatenate([ys[c][rows, :] for c in range(NT)], axis=1)
        x1 = x0 + ga * ((_ln(x0) * (1.0 + ca) + sa) * y)
        x1b[slot] = x1
        h2b[slot] = (_ln(x1) * (1.0 + cb) + sbb).astype(bf16)

    prep(0, 0)

    def ffn(r, _):
        slot = r % 2
        h2 = h2b[slot]
        x1 = x1b[slot]
        prep(jnp.minimum(r + 1, S // TM - 1), 1 - slot)
        o = b2
        for lo, hi in zip(FCUTS[:-1], FCUTS[1:]):
            h = lax.dot_general(h2, w1b[lo:hi, :], (((1,), (1,)), ((), ())), preferred_element_type=f32) + b1[:, lo:hi]
            g = jax.nn.gelu(h, approximate=True).astype(bf16)
            o = o + jnp.dot(g, w2b[lo:hi, :], preferred_element_type=f32)

        @pl.when(r >= 2)
        def _():
            out_copy(r - 2, slot).wait()
        ob[slot] = (x1 + gb * o).astype(bf16)
        out_copy(r, slot).start()
        return 0
    with jax.named_scope('ffn'):
        lax.fori_loop(0, S // TM, ffn, 0, unroll=1)
    out_copy(S // TM - 2, 0).wait()
    out_copy(S // TM - 1, 1).wait()


@jax.jit
def pallas_adaLN_cond__ssm_conv_h3__dense_activation_gelu__prompt_kernel(
    A_q, A_k, A_v, A_shift_k, A_ssm_k, A_ssm_D, B_x, B_w1, B_b1, B_w2, B_b2, c, w_mod,
):
    del B_x
    fwd, inv = _dft_consts()
    hbm = pl.BlockSpec(memory_space=pltpu.HBM)
    vm = pl.BlockSpec(memory_space=pltpu.VMEM)
    return pl.pallas_call(
        _kernel,
        in_specs=[hbm, hbm, hbm, vm, hbm, vm, hbm, vm, hbm, vm, vm, hbm, vm, vm],
        out_specs=hbm,
        out_shape=jax.ShapeDtypeStruct((1, S, D), bf16),
        scratch_shapes=[
            pltpu.VMEM((S, D), bf16),
            pltpu.VMEM((NT, S + HALO, 128), bf16),
            pltpu.VMEM((NT, S, 128), bf16),
            pltpu.VMEM((NT, 128, S), bf16),
            pltpu.VMEM((F, D), bf16),
            pltpu.VMEM((F, D), bf16),
            pltpu.VMEM((D, 6 * D), bf16),
            pltpu.VMEM((2, C, 128), f32),
            pltpu.VMEM((2, TM, D), bf16),
            pltpu.VMEM((2, TM, D), f32),
            pltpu.VMEM((2, TM, D), bf16),
            pltpu.SemaphoreType.DMA((3, NT)),
            pltpu.SemaphoreType.DMA((4,)),
            pltpu.SemaphoreType.DMA((2,)),
        ] + [pltpu.VMEM((S, 128), f32)] * (2 * NT)
          + [pltpu.VMEM((NC, 3, C, 128), f32)] * 4
          + [pltpu.VMEM((NC, 2 * C, 128), f32)] * 2,
        compiler_params=pltpu.CompilerParams(vmem_limit_bytes=100 * 1024 * 1024),
    )(A_q, A_k, A_v, A_shift_k.T, A_ssm_k, A_ssm_D, B_w1.T, B_b1,
      B_w2, B_b2, c, w_mod, jnp.asarray(fwd, bf16), jnp.asarray(inv, bf16))
```

```python
import numpy as np
import jax
import jax.numpy as jnp
from jax import lax
import jax.experimental.pallas as pl
import jax.experimental.pallas.tpu as pltpu

S, D, F = 2048, 640, 1728
C = 128
NC = S // C
NT = D // 128
HALO = 16
FCUTS = (0,1024,F)
TM = 256
f32, bf16 = jnp.float32, jnp.bfloat16


def _dft_consts():
    f = np.arange(C, dtype=np.float64)[:, None] + 0.5
    t = np.arange(C, dtype=np.float64)[None, :]
    th = 2.0 * np.pi * f * t / (2 * C)
    fwd = np.concatenate([np.cos(th), -np.sin(th)], axis=0)
    inv = np.concatenate([np.cos(th).T, -np.sin(th).T], axis=1) / C
    return fwd.astype(np.float32), inv.astype(np.float32)


def _ln(x):
    m = jnp.mean(x, axis=-1, keepdims=True)
    xc = x - m
    v = jnp.mean(xc * xc, axis=-1, keepdims=True)
    return xc * lax.rsqrt(v + 1e-5)


def _kernel(q_h, k_h, v_h, shk_ref, ssm_h, ssd_ref, w1_h, b1_ref, w2_h, b2_ref, c_ref, wm_h,
            fwd_ref, inv_ref, o_h,
            qb, kb, vb, sb, w1b, w2b, wmb, kprev, modb, ob, x1b, h2b, sem_in, sem_w, sem_o, *rest):
    kvs, ys = rest[:NT], rest[NT:2 * NT]
    xs, ks, zs = (rest[2 * NT + 2 * n:2 * NT + 2 * n + 2] for n in range(3))
    def slab(c):
        cols = pl.ds(c * 128, 128)
        return (pltpu.make_async_copy(k_h.at[0, :, cols], kb.at[c, pl.ds(HALO, S)], sem_in.at[0, c]),
                pltpu.make_async_copy(v_h.at[0, :, cols], vb.at[c], sem_in.at[1, c]),
                pltpu.make_async_copy(ssm_h.at[cols, :], sb.at[c], sem_in.at[2, c]))
    for c in range(NT):
        for cp in slab(c):
            cp.start()
    cp_wm = pltpu.make_async_copy(wm_h, wmb, sem_w.at[0])
    cp_q = pltpu.make_async_copy(q_h.at[0], qb, sem_w.at[1])
    cp_w1 = pltpu.make_async_copy(w1_h, w1b, sem_w.at[2])
    cp_w2 = pltpu.make_async_copy(w2_h, w2b, sem_w.at[3])

    for c in range(NT):
        kb[c, pl.ds(0, HALO), :] = jnp.zeros((HALO, 128), bf16)


    taps = shk_ref[...].astype(f32)
    ssd = ssd_ref[...].reshape(1, D).astype(f32)
    sigma = (1 - 2 * (lax.broadcasted_iota(jnp.int32, (C, 128), 0) & 1)).astype(f32)

    def aligned(i, n):
        return pl.ds(pl.multiple_of(i * n, n), n)

    def stage_a(c, j):
        slot = c % 2
        lo, hi = c * 128, (c + 1) * 128
        w = kb[c, pl.ds(pl.multiple_of(j * C, C), C + HALO), :].astype(f32)
        ksh = w[HALO:] * taps[0:1, lo:hi]
        for s in range(1, 4):
            ksh = ksh + w[HALO - s:HALO - s + C] * taps[s:s + 1, lo:hi]
        kv = ksh * vb[c, aligned(j, C), :].astype(f32)
        kvs[c][aligned(j, C), :] = kv
        fw = fwd_ref[...]
        xh = jnp.dot(fw, kv.astype(bf16), preferred_element_type=f32)
        a, b = xh[:C], xh[C:]
        xs[slot][j, 0] = a
        xs[slot][j, 1] = b
        xs[slot][j, 2] = a + b
        kh = lax.dot_general(fw, sb[c, :, aligned(j, C)], (((1,), (1,)), ((), ())),
                             preferred_element_type=f32)
        kc, kd = kh[:C], kh[C:]
        cc = kc - sigma * kprev[1]
        dd = kd + sigma * kprev[0]
        kprev[0] = kc
        kprev[1] = kd
        ks[slot][j, 0] = cc
        ks[slot][j, 1] = dd - cc
        ks[slot][j, 2] = cc + dd

    def stage_b(c, ft):
        slot = c % 2
        rows = aligned(ft, 8)
        IB = 4
        for i0 in range(0, NC, IB):
            acc = [[None] * 3 for _ in range(IB)]
            kreg = {}
            for j in range(i0 + IB):
                xa, xb, xab = (xs[slot][j, 2, rows, :], xs[slot][j, 0, rows, :], xs[slot][j, 1, rows, :])
                for ii in range(IB):
                    m = i0 + ii - j
                    if m < 0:
                        continue
                    if m not in kreg:
                        kreg[m] = tuple(ks[slot][m, p, rows, :] for p in range(3))
                    for p, xv in enumerate((xa, xb, xab)):
                        t = kreg[m][p] * xv
                        acc[ii][p] = t if acc[ii][p] is None else acc[ii][p] + t
                kreg.pop(i0 - j, None)
            for ii in range(IB):
                zs[slot][i0 + ii, rows, :] = acc[ii][0] - acc[ii][2]
                zs[slot][i0 + ii, pl.ds(pl.multiple_of(C + ft * 8, 8), 8), :] = acc[ii][0] + acc[ii][1]

    def stage_c(c, i):
        slot = c % 2
        y = jnp.dot(inv_ref[...], zs[slot][i].astype(bf16), preferred_element_type=f32)
        ys[c][aligned(i, C), :] = y + kvs[c][aligned(i, C), :] * ssd[:, c * 128:(c + 1) * 128]

    for c in range(-1, NT + 1):
        if 0 <= c + 1 < NT:
            if True:
                for cp in slab(c + 1):
                    cp.wait()
            for cp in {0: (cp_wm,), 1: (cp_q, cp_w1, cp_w2)}.get(c, ()):
                cp.start()
            kprev[...] = jnp.zeros_like(kprev)

        if c == NT - 1:
            cp_wm.wait()
            cv = c_ref[...].astype(f32)
            sc = jnp.broadcast_to((cv * jax.nn.sigmoid(cv)).astype(bf16), (8, D))

        def body(t, _, c=c):
            if c == NT - 1:
                cols = aligned(jnp.minimum(t, 14), 256)
                modb[:, cols] = jnp.dot(sc, wmb[:, cols], preferred_element_type=f32)
            if 0 <= c + 1 < NT:
                stage_a(c + 1, t)
            if 0 <= c < NT:
                stage_b(c, t)
            if 0 <= c - 1 < NT:
                stage_c(c - 1, t)
            return 0
        if True:
            lax.fori_loop(0, NC, body, 0, unroll=16)

    if True:
        mod = modb[0:1, :]
        sa, ca, ga, sbb, cb, gb = (mod[:, n * D:(n + 1) * D] for n in range(6))
        b1 = b1_ref[...].reshape(1, F).astype(f32)
        b2 = b2_ref[...].reshape(1, D).astype(f32)
        cp_q.wait()
        cp_w1.wait()
        cp_w2.wait()

    def out_copy(r, slot):
        return pltpu.make_async_copy(ob.at[slot], o_h.at[0, aligned(r, TM), :], sem_o.at[slot])

    def prep(r, slot):
        rows = aligned(r, TM)
        x0 = qb[rows, :].astype(f32)
        y = jnp.concatenate([ys[c][rows, :] for c in range(NT)], axis=1)
        x1 = x0 + ga * ((_ln(x0) * (1.0 + ca) + sa) * y)
        x1b[slot] = x1
        h2b[slot] = (_ln(x1) * (1.0 + cb) + sbb).astype(bf16)

    prep(0, 0)

    def ffn(r, _):
        slot = r % 2
        h2 = h2b[slot]
        x1 = x1b[slot]
        prep(jnp.minimum(r + 1, S // TM - 1), 1 - slot)
        o = b2
        for lo, hi in zip(FCUTS[:-1], FCUTS[1:]):
            h = lax.dot_general(h2, w1b[lo:hi, :], (((1,), (1,)), ((), ())), preferred_element_type=f32) + b1[:, lo:hi]
            g = jax.nn.gelu(h, approximate=True).astype(bf16)
            o = o + jnp.dot(g, w2b[lo:hi, :], preferred_element_type=f32)

        @pl.when(r >= 2)
        def _():
            out_copy(r - 2, slot).wait()
        ob[slot] = (x1 + gb * o).astype(bf16)
        out_copy(r, slot).start()
        return 0
    if True:
        lax.fori_loop(0, S // TM, ffn, 0, unroll=1)
    out_copy(S // TM - 2, 0).wait()
    out_copy(S // TM - 1, 1).wait()


@jax.jit
def pallas_adaLN_cond__ssm_conv_h3__dense_activation_gelu__prompt_kernel(
    A_q, A_k, A_v, A_shift_k, A_ssm_k, A_ssm_D, B_x, B_w1, B_b1, B_w2, B_b2, c, w_mod,
):
    del B_x
    fwd, inv = _dft_consts()
    hbm = pl.BlockSpec(memory_space=pltpu.HBM)
    vm = pl.BlockSpec(memory_space=pltpu.VMEM)
    return pl.pallas_call(
        _kernel,
        in_specs=[hbm, hbm, hbm, vm, hbm, vm, hbm, vm, hbm, vm, vm, hbm, vm, vm],
        out_specs=hbm,
        out_shape=jax.ShapeDtypeStruct((1, S, D), bf16),
        scratch_shapes=[
            pltpu.VMEM((S, D), bf16),
            pltpu.VMEM((NT, S + HALO, 128), bf16),
            pltpu.VMEM((NT, S, 128), bf16),
            pltpu.VMEM((NT, 128, S), bf16),
            pltpu.VMEM((F, D), bf16),
            pltpu.VMEM((F, D), bf16),
            pltpu.VMEM((D, 6 * D), bf16),
            pltpu.VMEM((2, C, 128), f32),
            pltpu.VMEM((8, 6 * D), f32),
            pltpu.VMEM((2, TM, D), bf16),
            pltpu.VMEM((2, TM, D), f32),
            pltpu.VMEM((2, TM, D), bf16),
            pltpu.SemaphoreType.DMA((3, NT)),
            pltpu.SemaphoreType.DMA((4,)),
            pltpu.SemaphoreType.DMA((2,)),
        ] + [pltpu.VMEM((S, 128), f32)] * (2 * NT)
          + [pltpu.VMEM((NC, 3, C, 128), f32)] * 4
          + [pltpu.VMEM((NC, 2 * C, 128), f32)] * 2,
        compiler_params=pltpu.CompilerParams(vmem_limit_bytes=100 * 1024 * 1024),
    )(A_q, A_k, A_v, A_shift_k.T, A_ssm_k, A_ssm_D, B_w1.T, B_b1,
      B_w2, B_b2, c, w_mod, jnp.asarray(fwd, bf16), jnp.asarray(inv, bf16))
```

```python
import numpy as np
import jax
import jax.numpy as jnp
from jax import lax
import jax.experimental.pallas as pl
import jax.experimental.pallas.tpu as pltpu

S, D, F = 2048, 640, 1728
C = 128
NC = S // C
NT = D // 128
HALO = 16
FCUTS = (0,1024,F)
TM = 256
f32, bf16 = jnp.float32, jnp.bfloat16


def _dft_consts():
    f = np.arange(C, dtype=np.float64)[:, None] + 0.5
    t = np.arange(C, dtype=np.float64)[None, :]
    th = 2.0 * np.pi * f * t / (2 * C)
    fwd = np.concatenate([np.cos(th), -np.sin(th)], axis=0)
    inv = np.concatenate([np.cos(th).T, -np.sin(th).T], axis=1) / C
    return fwd.astype(np.float32), inv.astype(np.float32)


def _ln(x):
    m = jnp.mean(x, axis=-1, keepdims=True)
    xc = x - m
    v = jnp.mean(xc * xc, axis=-1, keepdims=True)
    return xc * lax.rsqrt(v + 1e-5)


def _kernel(q_h, k_h, v_h, shk_ref, ssm_h, ssd_ref, w1_h, b1_ref, w2_h, b2_ref, c_ref, wm_h,
            fwd_ref, inv_ref, o_h,
            qb, kb, vb, sb, w1b, w2b, wmb, kprev, modb, ob, x1b, h2b, sem_in, sem_w, sem_o, *rest):
    ys = rest[:NT]
    xs, ks, zs = (rest[NT + 2 * n:NT + 2 * n + 2] for n in range(3))
    def slab(c):
        cols = pl.ds(c * 128, 128)
        return (pltpu.make_async_copy(k_h.at[0, :, cols], kb.at[c, pl.ds(HALO, S)], sem_in.at[0, c]),
                pltpu.make_async_copy(v_h.at[0, :, cols], vb.at[c], sem_in.at[1, c]),
                pltpu.make_async_copy(ssm_h.at[cols, :], sb.at[c], sem_in.at[2, c]))
    for c in range(NT):
        for cp in slab(c):
            cp.start()
    cp_wm = pltpu.make_async_copy(wm_h, wmb, sem_w.at[0])
    cp_q = pltpu.make_async_copy(q_h.at[0], qb, sem_w.at[1])
    cp_w1 = pltpu.make_async_copy(w1_h, w1b, sem_w.at[2])
    cp_w2 = pltpu.make_async_copy(w2_h, w2b, sem_w.at[3])

    for c in range(NT):
        kb[c, pl.ds(0, HALO), :] = jnp.zeros((HALO, 128), bf16)


    taps = shk_ref[...].astype(f32)
    ssd = ssd_ref[...].reshape(1, D).astype(f32)
    sigma = (1 - 2 * (lax.broadcasted_iota(jnp.int32, (C, 128), 0) & 1)).astype(f32)

    def aligned(i, n):
        return pl.ds(i * n if isinstance(i, int) else pl.multiple_of(i * n, n), n)

    def stage_a(c, j):
        slot = c % 2
        lo, hi = c * 128, (c + 1) * 128
        w = kb[c, pl.ds(j * C, C + HALO), :].astype(f32)
        ksh = w[HALO:] * taps[0:1, lo:hi]
        for s in range(1, 4):
            ksh = ksh + w[HALO - s:HALO - s + C] * taps[s:s + 1, lo:hi]
        kv = ksh * vb[c, aligned(j, C), :].astype(f32)
        fw = fwd_ref[...]
        xh = jnp.dot(fw, kv.astype(bf16), preferred_element_type=f32)
        a, b = xh[:C], xh[C:]
        xs[slot][j, 0] = a
        xs[slot][j, 1] = b
        xs[slot][j, 2] = a + b
        kh = lax.dot_general(fw, sb[c, :, aligned(j, C)], (((1,), (1,)), ((), ())),
                             preferred_element_type=f32)
        kc, kd = kh[:C], kh[C:]
        if j == 0:
            kc = kc + ssd[:, lo:hi]
            cc, dd = kc, kd
        else:
            cc = kc - sigma * kprev[1]
            dd = kd + sigma * kprev[0]
        kprev[0] = kc
        kprev[1] = kd
        ks[slot][j, 0] = cc
        ks[slot][j, 1] = dd - cc
        ks[slot][j, 2] = cc + dd

    def stage_b(c, ft):
        slot = c % 2
        rows = aligned(ft, 8)
        IB = 4
        for i0 in range(0, NC, IB):
            acc = [[None] * 3 for _ in range(IB)]
            kreg = {}
            for j in range(i0 + IB):
                xa, xb, xab = (xs[slot][j, 2, rows, :], xs[slot][j, 0, rows, :], xs[slot][j, 1, rows, :])
                for ii in range(IB):
                    m = i0 + ii - j
                    if m < 0:
                        continue
                    if m not in kreg:
                        kreg[m] = tuple(ks[slot][m, p, rows, :] for p in range(3))
                    for p, xv in enumerate((xa, xb, xab)):
                        t = kreg[m][p] * xv
                        acc[ii][p] = t if acc[ii][p] is None else acc[ii][p] + t
                kreg.pop(i0 - j, None)
            for ii in range(IB):
                zs[slot][i0 + ii, rows, :] = acc[ii][0] - acc[ii][2]
                zs[slot][i0 + ii, pl.ds(C + ft * 8, 8), :] = acc[ii][0] + acc[ii][1]

    def stage_c(c, i):
        slot = c % 2
        y = jnp.dot(inv_ref[...], zs[slot][i].astype(bf16), preferred_element_type=f32)
        ys[c][aligned(i, C), :] = y

    for c in range(-1, NT + 1):
        if 0 <= c + 1 < NT:
            if True:
                for cp in slab(c + 1):
                    cp.wait()
            for cp in {0: (cp_wm,), 1: (cp_q, cp_w1, cp_w2)}.get(c, ()):
                cp.start()

        if c == NT - 1:
            cp_wm.wait()
            cv = c_ref[...].astype(f32)
            sc = jnp.broadcast_to((cv * jax.nn.sigmoid(cv)).astype(bf16), (8, D))

        def body(t, _, c=c):
            if c == NT - 1 and t < 15:
                cols = aligned(t, 256)
                modb[:, cols] = jnp.dot(sc, wmb[:, cols], preferred_element_type=f32)
            if 0 <= c + 1 < NT:
                stage_a(c + 1, t)
            if 0 <= c < NT:
                stage_b(c, t)
            if 0 <= c - 1 < NT:
                stage_c(c - 1, t)
            return 0
        if True:
            for t in range(NC):
                body(t, 0)

    if True:
        mod = modb[0:1, :]
        sa, ca, ga, sbb, cb, gb = (mod[:, n * D:(n + 1) * D] for n in range(6))
        b1 = b1_ref[...].reshape(1, F).astype(f32)
        b2 = b2_ref[...].reshape(1, D).astype(f32)
        cp_q.wait()
        cp_w1.wait()
        cp_w2.wait()

    def out_copy(r, slot):
        return pltpu.make_async_copy(ob.at[slot], o_h.at[0, aligned(r, TM), :], sem_o.at[slot])

    def prep(r, slot):
        rows = aligned(r, TM)
        x0 = qb[rows, :].astype(f32)
        y = jnp.concatenate([ys[c][rows, :] for c in range(NT)], axis=1)
        x1 = x0 + ga * ((_ln(x0) * (1.0 + ca) + sa) * y)
        x1b[slot] = x1
        h2b[slot] = (_ln(x1) * (1.0 + cb) + sbb).astype(bf16)

    prep(0, 0)

    def ffn(r, _):
        slot = r % 2
        h2 = h2b[slot]
        x1 = x1b[slot]
        prep(jnp.minimum(r + 1, S // TM - 1), 1 - slot)
        o = b2
        for lo, hi in zip(FCUTS[:-1], FCUTS[1:]):
            h = lax.dot_general(h2, w1b[lo:hi, :], (((1,), (1,)), ((), ())), preferred_element_type=f32) + b1[:, lo:hi]
            g = jax.nn.gelu(h, approximate=True).astype(bf16)
            o = o + jnp.dot(g, w2b[lo:hi, :], preferred_element_type=f32)

        @pl.when(r >= 2)
        def _():
            out_copy(r - 2, slot).wait()
        ob[slot] = (x1 + gb * o).astype(bf16)
        out_copy(r, slot).start()
        return 0
    if True:
        lax.fori_loop(0, S // TM, ffn, 0, unroll=1)
    out_copy(S // TM - 2, 0).wait()
    out_copy(S // TM - 1, 1).wait()


@jax.jit
def pallas_adaLN_cond__ssm_conv_h3__dense_activation_gelu__prompt_kernel(
    A_q, A_k, A_v, A_shift_k, A_ssm_k, A_ssm_D, B_x, B_w1, B_b1, B_w2, B_b2, c, w_mod,
):
    del B_x
    fwd, inv = _dft_consts()
    hbm = pl.BlockSpec(memory_space=pltpu.HBM)
    vm = pl.BlockSpec(memory_space=pltpu.VMEM)
    return pl.pallas_call(
        _kernel,
        in_specs=[hbm, hbm, hbm, vm, hbm, vm, hbm, vm, hbm, vm, vm, hbm, vm, vm],
        out_specs=hbm,
        out_shape=jax.ShapeDtypeStruct((1, S, D), bf16),
        scratch_shapes=[
            pltpu.VMEM((S, D), bf16),
            pltpu.VMEM((NT, S + HALO, 128), bf16),
            pltpu.VMEM((NT, S, 128), bf16),
            pltpu.VMEM((NT, 128, S), bf16),
            pltpu.VMEM((F, D), bf16),
            pltpu.VMEM((F, D), bf16),
            pltpu.VMEM((D, 6 * D), bf16),
            pltpu.VMEM((2, C, 128), f32),
            pltpu.VMEM((8, 6 * D), f32),
            pltpu.VMEM((2, TM, D), bf16),
            pltpu.VMEM((2, TM, D), f32),
            pltpu.VMEM((2, TM, D), bf16),
            pltpu.SemaphoreType.DMA((3, NT)),
            pltpu.SemaphoreType.DMA((4,)),
            pltpu.SemaphoreType.DMA((2,)),
        ] + [pltpu.VMEM((S, 128), f32)] * NT
          + [pltpu.VMEM((NC, 3, C, 128), f32)] * 4
          + [pltpu.VMEM((NC, 2 * C, 128), f32)] * 2,
        compiler_params=pltpu.CompilerParams(vmem_limit_bytes=100 * 1024 * 1024),
    )(A_q, A_k, A_v, A_shift_k.T, A_ssm_k, A_ssm_D, B_w1.T, B_b1,
      B_w2, B_b2, c, w_mod, jnp.asarray(fwd, bf16), jnp.asarray(inv, bf16))
```

```python
import numpy as np
import jax
import jax.numpy as jnp
from jax import lax
import jax.experimental.pallas as pl
import jax.experimental.pallas.tpu as pltpu

S, D, F = 2048, 640, 1728
C = 128
NC = S // C
NT = D // 128
HALO = 16
FCUTS = (0,1024,F)
TM = 256
f32, bf16 = jnp.float32, jnp.bfloat16


def _dft_consts():
    f = np.arange(C, dtype=np.float64)[:, None] + 0.5
    t = np.arange(C, dtype=np.float64)[None, :]
    th = 2.0 * np.pi * f * t / (2 * C)
    fwd = np.concatenate([np.cos(th), -np.sin(th)], axis=0)
    inv = np.concatenate([np.cos(th).T, -np.sin(th).T], axis=1) / C
    return fwd.astype(np.float32), inv.astype(np.float32)


def _ln(x):
    m = jnp.mean(x, axis=-1, keepdims=True)
    xc = x - m
    v = jnp.mean(xc * xc, axis=-1, keepdims=True)
    return xc * lax.rsqrt(v + 1e-5)


def _kernel(q_h, k_h, v_h, shk_ref, ssm_h, ssd_ref, w1_h, b1_ref, w2_h, b2_ref, c_ref, wm_h,
            fwd_ref, inv_ref, o_h,
            qb, kb, vb, sb, w1b, w2b, wmb, kprev, modb, ob, x1b, h2b, sem_in, sem_w, sem_o, *rest):
    ys = rest[:NT]
    xs, ks, zs = (rest[NT + 2 * n:NT + 2 * n + 2] for n in range(3))
    def slab(c):
        cols = pl.ds(c * 128, 128)
        return (pltpu.make_async_copy(k_h.at[0, :, cols], kb.at[c, pl.ds(HALO, S)], sem_in.at[0, c]),
                pltpu.make_async_copy(v_h.at[0, :, cols], vb.at[c], sem_in.at[1, c]),
                pltpu.make_async_copy(ssm_h.at[cols, :], sb.at[c], sem_in.at[2, c]))
    for c in range(NT):
        for cp in slab(c):
            cp.start()
    cp_wm = pltpu.make_async_copy(wm_h, wmb, sem_w.at[0])
    cp_q = pltpu.make_async_copy(q_h.at[0], qb, sem_w.at[1])
    cp_w1 = pltpu.make_async_copy(w1_h, w1b, sem_w.at[2])
    cp_w2 = pltpu.make_async_copy(w2_h, w2b, sem_w.at[3])

    for c in range(NT):
        kb[c, pl.ds(0, HALO), :] = jnp.zeros((HALO, 128), bf16)


    taps = shk_ref[...].astype(f32)
    ssd = ssd_ref[...].reshape(1, D).astype(f32)
    sigma = (1 - 2 * (lax.broadcasted_iota(jnp.int32, (C, 128), 0) & 1)).astype(f32)

    def aligned(i, n):
        return pl.ds(i * n if isinstance(i, int) else pl.multiple_of(i * n, n), n)

    def stage_a(c, j):
        slot = c % 2
        lo, hi = c * 128, (c + 1) * 128
        w = kb[c, pl.ds(j * C, C + HALO), :].astype(f32)
        ksh = w[HALO:] * taps[0:1, lo:hi]
        for s in range(1, 4):
            ksh = ksh + w[HALO - s:HALO - s + C] * taps[s:s + 1, lo:hi]
        kv = ksh * vb[c, aligned(j, C), :].astype(f32)
        fw = fwd_ref[...]
        xh = jnp.dot(fw, kv.astype(bf16), preferred_element_type=f32)
        a, b = xh[:C], xh[C:]
        xs[slot][j, 0] = a
        xs[slot][j, 1] = b
        xs[slot][j, 2] = a + b
        kh = lax.dot_general(fw, sb[c, :, aligned(j, C)], (((1,), (1,)), ((), ())),
                             preferred_element_type=f32)
        kc, kd = kh[:C], kh[C:]
        if j == 0:
            kc = kc + ssd[:, lo:hi]
            cc, dd = kc, kd
        else:
            cc = kc - sigma * kprev[1]
            dd = kd + sigma * kprev[0]
        kprev[0] = kc
        kprev[1] = kd
        ks[slot][j, 0] = cc
        ks[slot][j, 1] = dd - cc
        ks[slot][j, 2] = cc + dd

    def stage_b(c, ft):
        slot = c % 2
        rows = aligned(ft, 8)
        IB = 4
        for i0 in range(0, NC, IB):
            acc = [[None] * 3 for _ in range(IB)]
            kreg = {}
            for j in range(i0 + IB):
                xa, xb, xab = (xs[slot][j, 2, rows, :], xs[slot][j, 0, rows, :], xs[slot][j, 1, rows, :])
                for ii in range(IB):
                    m = i0 + ii - j
                    if m < 0:
                        continue
                    if m not in kreg:
                        kreg[m] = tuple(ks[slot][m, p, rows, :] for p in range(3))
                    for p, xv in enumerate((xa, xb, xab)):
                        t = kreg[m][p] * xv
                        acc[ii][p] = t if acc[ii][p] is None else acc[ii][p] + t
                kreg.pop(i0 - j, None)
            for ii in range(IB):
                zs[slot][i0 + ii, rows, :] = acc[ii][0] - acc[ii][2]
                zs[slot][i0 + ii, pl.ds(C + ft * 8, 8), :] = acc[ii][0] + acc[ii][1]

    def stage_c(c, i):
        slot = c % 2
        y = jnp.dot(inv_ref[...], zs[slot][i].astype(bf16), preferred_element_type=f32)
        ys[c][aligned(i, C), :] = y

    for c in range(-1, NT + 1):
        if 0 <= c + 1 < NT:
            if True:
                for cp in slab(c + 1):
                    cp.wait()
            for cp in {0: (cp_wm,), 1: (cp_q, cp_w1, cp_w2)}.get(c, ()):
                cp.start()

        if c == NT - 1:
            cp_wm.wait()
            cv = c_ref[...].astype(f32)
            sc = jnp.broadcast_to((cv * jax.nn.sigmoid(cv)).astype(bf16), (8, D))

        def body(t, _, c=c):
            if c == NT - 1 and t < 15:
                cols = aligned(t, 256)
                modb[:, cols] = jnp.dot(sc, wmb[:, cols], preferred_element_type=f32)
            if 0 <= c + 1 < NT:
                stage_a(c + 1, t)
            if 0 <= c < NT:
                stage_b(c, t)
            if 0 <= c - 1 < NT:
                stage_c(c - 1, t)
            return 0
        if True:
            for t in range(NC):
                body(t, 0)

    if True:
        mod = modb[0:1, :]
        sa, ca, ga, sbb, cb, gb = (mod[:, n * D:(n + 1) * D] for n in range(6))
        b1 = b1_ref[...].reshape(1, F).astype(f32)
        b2 = b2_ref[...].reshape(1, D).astype(f32)
        cp_q.wait()
        cp_w1.wait()
        cp_w2.wait()

    def out_copy(r, slot):
        return pltpu.make_async_copy(ob.at[slot], o_h.at[0, aligned(r, TM), :], sem_o.at[slot])

    def prep(r, slot):
        rows = aligned(r, TM)
        x0 = qb[rows, :].astype(f32)
        y = jnp.concatenate([ys[c][rows, :] for c in range(NT)], axis=1)
        x1 = x0 + ga * ((_ln(x0) * (1.0 + ca) + sa) * y)
        x1b[slot] = x1
        hn = (_ln(x1) * (1.0 + cb) + sbb).astype(bf16)
        h2b[slot] = hn
        return hn

    prep(0, 0)

    def ffn(r, _):
        slot = r % 2
        h2 = h2b[slot]
        x1 = x1b[slot]
        hn = prep(jnp.minimum(r + 1, S // TM - 1), 1 - slot)
        o = b2
        for lo, hi in zip(FCUTS[:-1], FCUTS[1:]):
            h = lax.dot_general(h2, w1b[lo:hi, :], (((1,), (1,)), ((), ())), preferred_element_type=f32) + b1[:, lo:hi]
            g = jax.nn.gelu(h, approximate=True).astype(bf16)
            if lo == 0:
                h2 = jnp.where(r < 0, hn, h2)
            o = o + jnp.dot(g, w2b[lo:hi, :], preferred_element_type=f32)

        @pl.when(r >= 2)
        def _():
            out_copy(r - 2, slot).wait()
        ob[slot] = (x1 + gb * o).astype(bf16)
        out_copy(r, slot).start()
        return 0
    if True:
        lax.fori_loop(0, S // TM, ffn, 0, unroll=1)
    out_copy(S // TM - 2, 0).wait()
    out_copy(S // TM - 1, 1).wait()


@jax.jit
def pallas_adaLN_cond__ssm_conv_h3__dense_activation_gelu__prompt_kernel(
    A_q, A_k, A_v, A_shift_k, A_ssm_k, A_ssm_D, B_x, B_w1, B_b1, B_w2, B_b2, c, w_mod,
):
    del B_x
    fwd, inv = _dft_consts()
    hbm = pl.BlockSpec(memory_space=pltpu.HBM)
    vm = pl.BlockSpec(memory_space=pltpu.VMEM)
    return pl.pallas_call(
        _kernel,
        in_specs=[hbm, hbm, hbm, vm, hbm, vm, hbm, vm, hbm, vm, vm, hbm, vm, vm],
        out_specs=hbm,
        out_shape=jax.ShapeDtypeStruct((1, S, D), bf16),
        scratch_shapes=[
            pltpu.VMEM((S, D), bf16),
            pltpu.VMEM((NT, S + HALO, 128), bf16),
            pltpu.VMEM((NT, S, 128), bf16),
            pltpu.VMEM((NT, 128, S), bf16),
            pltpu.VMEM((F, D), bf16),
            pltpu.VMEM((F, D), bf16),
            pltpu.VMEM((D, 6 * D), bf16),
            pltpu.VMEM((2, C, 128), f32),
            pltpu.VMEM((8, 6 * D), f32),
            pltpu.VMEM((2, TM, D), bf16),
            pltpu.VMEM((2, TM, D), f32),
            pltpu.VMEM((2, TM, D), bf16),
            pltpu.SemaphoreType.DMA((3, NT)),
            pltpu.SemaphoreType.DMA((4,)),
            pltpu.SemaphoreType.DMA((2,)),
        ] + [pltpu.VMEM((S, 128), f32)] * NT
          + [pltpu.VMEM((NC, 3, C, 128), f32)] * 4
          + [pltpu.VMEM((NC, 2 * C, 128), f32)] * 2,
        compiler_params=pltpu.CompilerParams(vmem_limit_bytes=100 * 1024 * 1024),
    )(A_q, A_k, A_v, A_shift_k.T, A_ssm_k, A_ssm_D, B_w1.T, B_b1,
      B_w2, B_b2, c, w_mod, jnp.asarray(fwd, bf16), jnp.asarray(inv, bf16))
```

```python
import numpy as np
import jax
import jax.numpy as jnp
from jax import lax
import jax.experimental.pallas as pl
import jax.experimental.pallas.tpu as pltpu

S, D, F = 2048, 640, 1728
C = 128
NC = S // C
NT = D // 128
HALO = 16
FCUTS = (0,1024,F)
TM = 256
f32, bf16 = jnp.float32, jnp.bfloat16


def _dft_consts():
    f = np.arange(C, dtype=np.float64)[:, None] + 0.5
    t = np.arange(C, dtype=np.float64)[None, :]
    th = 2.0 * np.pi * f * t / (2 * C)
    fwd = np.concatenate([np.cos(th), -np.sin(th)], axis=0)
    inv = np.concatenate([np.cos(th).T, -np.sin(th).T], axis=1) / C
    return fwd.astype(np.float32), inv.astype(np.float32)


def _ln(x):
    m = jnp.mean(x, axis=-1, keepdims=True)
    xc = x - m
    v = jnp.mean(xc * xc, axis=-1, keepdims=True)
    return xc * lax.rsqrt(v + 1e-5)


def _kernel(q_h, k_h, v_h, shk_ref, ssm_h, ssd_ref, w1_h, b1_ref, w2_h, b2_ref, c_ref, wm_h,
            fwd_ref, inv_ref, o_h,
            qb, kb, vb, sb, w1b, w2b, wmb, kprev, modb, ob, x1b, h2b, sem_in, sem_w, sem_o, *rest):
    ys = rest[:NT]
    kfs = rest[NT + 6:NT + 8]
    xs, ks, zs = (rest[NT + 2 * n:NT + 2 * n + 2] for n in range(3))
    def slab(c):
        cols = pl.ds(c * 128, 128)
        return (pltpu.make_async_copy(k_h.at[0, :, cols], kb.at[c, pl.ds(HALO, S)], sem_in.at[0, c]),
                pltpu.make_async_copy(v_h.at[0, :, cols], vb.at[c], sem_in.at[1, c]),
                pltpu.make_async_copy(ssm_h.at[cols, :], sb.at[c], sem_in.at[2, c]))
    for c in range(NT):
        for cp in slab(c):
            cp.start()
    cp_wm = pltpu.make_async_copy(wm_h, wmb, sem_w.at[0])
    cp_q = pltpu.make_async_copy(q_h.at[0], qb, sem_w.at[1])
    cp_w1 = pltpu.make_async_copy(w1_h, w1b, sem_w.at[2])
    cp_w2 = pltpu.make_async_copy(w2_h, w2b, sem_w.at[3])

    for c in range(NT):
        kb[c, pl.ds(0, HALO), :] = jnp.zeros((HALO, 128), bf16)


    taps = shk_ref[...].astype(f32)
    ssd = ssd_ref[...].reshape(1, D).astype(f32)
    sigma = (1 - 2 * (lax.broadcasted_iota(jnp.int32, (C, 128), 0) & 1)).astype(f32)

    def aligned(i, n):
        return pl.ds(i * n if isinstance(i, int) else pl.multiple_of(i * n, n), n)

    def stage_a(c, j):
        slot = c % 2
        lo, hi = c * 128, (c + 1) * 128
        w = kb[c, pl.ds(HALO + j * C, C), :].astype(f32)
        kf = kfs[slot]
        if j == 0:
            kf[pl.ds(0, 8), :] = jnp.zeros((8, 128), f32)
        kf[pl.ds(8 + j * C, C), :] = w
        ksh = w * taps[0:1, lo:hi]
        for s in range(1, 4):
            ksh = ksh + kf[pl.ds(8 + j * C - s, C), :] * taps[s:s + 1, lo:hi]
        kv = ksh * vb[c, aligned(j, C), :].astype(f32)
        fw = fwd_ref[...]
        xh = jnp.dot(fw, kv.astype(bf16), preferred_element_type=f32)
        a, b = xh[:C], xh[C:]
        xs[slot][j, 0] = a
        xs[slot][j, 1] = b
        xs[slot][j, 2] = a + b
        kh = lax.dot_general(fw, sb[c, :, aligned(j, C)], (((1,), (1,)), ((), ())),
                             preferred_element_type=f32)
        kc, kd = kh[:C], kh[C:]
        if j == 0:
            kc = kc + ssd[:, lo:hi]
            cc, dd = kc, kd
        else:
            cc = kc - sigma * kprev[1]
            dd = kd + sigma * kprev[0]
        kprev[0] = kc
        kprev[1] = kd
        ks[slot][j, 0] = cc
        ks[slot][j, 1] = dd - cc
        ks[slot][j, 2] = cc + dd

    def stage_b(c, ft):
        slot = c % 2
        rows = aligned(ft, 8)
        IB = 4
        for i0 in range(0, NC, IB):
            acc = [[None] * 3 for _ in range(IB)]
            kreg = {}
            for j in range(i0 + IB):
                xa, xb, xab = (xs[slot][j, 2, rows, :], xs[slot][j, 0, rows, :], xs[slot][j, 1, rows, :])
                for ii in range(IB):
                    m = i0 + ii - j
                    if m < 0:
                        continue
                    if m not in kreg:
                        kreg[m] = tuple(ks[slot][m, p, rows, :] for p in range(3))
                    for p, xv in enumerate((xa, xb, xab)):
                        t = kreg[m][p] * xv
                        acc[ii][p] = t if acc[ii][p] is None else acc[ii][p] + t
                kreg.pop(i0 - j, None)
            for ii in range(IB):
                zs[slot][i0 + ii, rows, :] = acc[ii][0] - acc[ii][2]
                zs[slot][i0 + ii, pl.ds(C + ft * 8, 8), :] = acc[ii][0] + acc[ii][1]

    def stage_c(c, i):
        slot = c % 2
        y = jnp.dot(inv_ref[...], zs[slot][i].astype(bf16), preferred_element_type=f32)
        ys[c][aligned(i, C), :] = y

    for c in range(-1, NT + 1):
        if 0 <= c + 1 < NT:
            if True:
                for cp in slab(c + 1):
                    cp.wait()
            for cp in {0: (cp_wm,), 1: (cp_q, cp_w1, cp_w2)}.get(c, ()):
                cp.start()

        if c == NT - 1:
            cp_wm.wait()
            cv = c_ref[...].astype(f32)
            sc = jnp.broadcast_to((cv * jax.nn.sigmoid(cv)).astype(bf16), (8, D))

        def body(t, _, c=c):
            if c == NT - 1 and t < 15:
                cols = aligned(t, 256)
                modb[:, cols] = jnp.dot(sc, wmb[:, cols], preferred_element_type=f32)
            if 0 <= c + 1 < NT:
                stage_a(c + 1, t)
            if 0 <= c < NT:
                stage_b(c, t)
            if 0 <= c - 1 < NT:
                stage_c(c - 1, t)
            return 0
        if True:
            for t in range(NC):
                body(t, 0)

    if True:
        mod = modb[0:1, :]
        sa, ca, ga, sbb, cb, gb = (mod[:, n * D:(n + 1) * D] for n in range(6))
        b1 = b1_ref[...].reshape(1, F).astype(f32)
        b2 = b2_ref[...].reshape(1, D).astype(f32)
        cp_q.wait()
        cp_w1.wait()
        cp_w2.wait()

    def out_copy(r, slot):
        return pltpu.make_async_copy(ob.at[slot], o_h.at[0, aligned(r, TM), :], sem_o.at[slot])

    def prep(r, slot):
        rows = aligned(r, TM)
        x0 = qb[rows, :].astype(f32)
        y = jnp.concatenate([ys[c][rows, :] for c in range(NT)], axis=1)
        x1 = x0 + ga * ((_ln(x0) * (1.0 + ca) + sa) * y)
        x1b[slot] = x1
        hn = (_ln(x1) * (1.0 + cb) + sbb).astype(bf16)
        h2b[slot] = hn
        return hn

    prep(0, 0)

    def ffn(r, _):
        slot = r % 2
        h2 = h2b[slot]
        x1 = x1b[slot]
        hn = prep(jnp.minimum(r + 1, S // TM - 1), 1 - slot)
        o = b2
        for lo, hi in zip(FCUTS[:-1], FCUTS[1:]):
            h = lax.dot_general(h2, w1b[lo:hi, :], (((1,), (1,)), ((), ())), preferred_element_type=f32) + b1[:, lo:hi]
            g = jax.nn.gelu(h, approximate=True).astype(bf16)
            if lo == 0:
                h2 = jnp.where(r < 0, hn, h2)
            o = o + jnp.dot(g, w2b[lo:hi, :], preferred_element_type=f32)

        @pl.when(r >= 2)
        def _():
            out_copy(r - 2, slot).wait()
        ob[slot] = (x1 + gb * o).astype(bf16)
        out_copy(r, slot).start()
        return 0
    if True:
        lax.fori_loop(0, S // TM, ffn, 0, unroll=1)
    out_copy(S // TM - 2, 0).wait()
    out_copy(S // TM - 1, 1).wait()


@jax.jit
def pallas_adaLN_cond__ssm_conv_h3__dense_activation_gelu__prompt_kernel(
    A_q, A_k, A_v, A_shift_k, A_ssm_k, A_ssm_D, B_x, B_w1, B_b1, B_w2, B_b2, c, w_mod,
):
    del B_x
    fwd, inv = _dft_consts()
    hbm = pl.BlockSpec(memory_space=pltpu.HBM)
    vm = pl.BlockSpec(memory_space=pltpu.VMEM)
    return pl.pallas_call(
        _kernel,
        in_specs=[hbm, hbm, hbm, vm, hbm, vm, hbm, vm, hbm, vm, vm, hbm, vm, vm],
        out_specs=hbm,
        out_shape=jax.ShapeDtypeStruct((1, S, D), bf16),
        scratch_shapes=[
            pltpu.VMEM((S, D), bf16),
            pltpu.VMEM((NT, S + HALO, 128), bf16),
            pltpu.VMEM((NT, S, 128), bf16),
            pltpu.VMEM((NT, 128, S), bf16),
            pltpu.VMEM((F, D), bf16),
            pltpu.VMEM((F, D), bf16),
            pltpu.VMEM((D, 6 * D), bf16),
            pltpu.VMEM((2, C, 128), f32),
            pltpu.VMEM((8, 6 * D), f32),
            pltpu.VMEM((2, TM, D), bf16),
            pltpu.VMEM((2, TM, D), f32),
            pltpu.VMEM((2, TM, D), bf16),
            pltpu.SemaphoreType.DMA((3, NT)),
            pltpu.SemaphoreType.DMA((4,)),
            pltpu.SemaphoreType.DMA((2,)),
        ] + [pltpu.VMEM((S, 128), f32)] * NT
          + [pltpu.VMEM((NC, 3, C, 128), f32)] * 4
          + [pltpu.VMEM((NC, 2 * C, 128), f32)] * 2
          + [pltpu.VMEM((8 + S, 128), f32)] * 2,
        compiler_params=pltpu.CompilerParams(vmem_limit_bytes=100 * 1024 * 1024),
    )(A_q, A_k, A_v, A_shift_k.T, A_ssm_k, A_ssm_D, B_w1.T, B_b1,
      B_w2, B_b2, c, w_mod, jnp.asarray(fwd, bf16), jnp.asarray(inv, bf16))
```

```python
import numpy as np
import jax
import jax.numpy as jnp
from jax import lax
import jax.experimental.pallas as pl
import jax.experimental.pallas.tpu as pltpu

S, D, F = 2048, 640, 1728
C = 128
NC = S // C
NT = D // 128
HALO = 16
FCUTS = (0,1024,F)
TM = 256
f32, bf16 = jnp.float32, jnp.bfloat16


def _dft_consts():
    f = np.arange(C, dtype=np.float64)[:, None] + 0.5
    t = np.arange(C, dtype=np.float64)[None, :]
    th = 2.0 * np.pi * f * t / (2 * C)
    fwd = np.concatenate([np.cos(th), -np.sin(th)], axis=0)
    inv = np.concatenate([np.cos(th).T, -np.sin(th).T], axis=1) / C
    return fwd.astype(np.float32), inv.astype(np.float32)


def _ln(x):
    m = jnp.mean(x, axis=-1, keepdims=True)
    xc = x - m
    v = jnp.mean(xc * xc, axis=-1, keepdims=True)
    return xc * lax.rsqrt(v + 1e-5)


def _kernel(q_h, k_h, v_h, shk_ref, ssm_h, ssd_ref, w1_h, b1_ref, w2_h, b2_ref, c_ref, wm_h,
            fwd_ref, inv_ref, o_h,
            qb, kb, vb, sb, w1b, w2b, wmb, kprev, modb, ob, x1a, x1c, h2a, h2c, sem_in, sem_w, sem_o, *rest):
    ys = rest[:NT]
    kfs = rest[NT + 6:NT + 8]
    xs, ks, zs = (rest[NT + 2 * n:NT + 2 * n + 2] for n in range(3))
    def slab(c):
        cols = pl.ds(c * 128, 128)
        return (pltpu.make_async_copy(k_h.at[0, :, cols], kb.at[c, pl.ds(HALO, S)], sem_in.at[0, c]),
                pltpu.make_async_copy(v_h.at[0, :, cols], vb.at[c], sem_in.at[1, c]),
                pltpu.make_async_copy(ssm_h.at[cols, :], sb.at[c], sem_in.at[2, c]))
    for c in range(NT):
        for cp in slab(c):
            cp.start()
    cp_wm = pltpu.make_async_copy(wm_h, wmb, sem_w.at[0])
    cp_q = pltpu.make_async_copy(q_h.at[0], qb, sem_w.at[1])
    cp_w1 = pltpu.make_async_copy(w1_h, w1b, sem_w.at[2])
    cp_w2 = pltpu.make_async_copy(w2_h, w2b, sem_w.at[3])

    for c in range(NT):
        kb[c, pl.ds(0, HALO), :] = jnp.zeros((HALO, 128), bf16)


    taps = shk_ref[...].astype(f32)
    ssd = ssd_ref[...].reshape(1, D).astype(f32)
    sigma = (1 - 2 * (lax.broadcasted_iota(jnp.int32, (C, 128), 0) & 1)).astype(f32)

    def aligned(i, n):
        return pl.ds(i * n if isinstance(i, int) else pl.multiple_of(i * n, n), n)

    def stage_a(c, j):
        slot = c % 2
        lo, hi = c * 128, (c + 1) * 128
        w = kb[c, pl.ds(HALO + j * C, C), :].astype(f32)
        kf = kfs[slot]
        if j == 0:
            kf[pl.ds(0, 8), :] = jnp.zeros((8, 128), f32)
        kf[pl.ds(8 + j * C, C), :] = w
        ksh = w * taps[0:1, lo:hi]
        for s in range(1, 4):
            ksh = ksh + kf[pl.ds(8 + j * C - s, C), :] * taps[s:s + 1, lo:hi]
        kv = ksh * vb[c, aligned(j, C), :].astype(f32)
        fw = fwd_ref[...]
        xh = jnp.dot(fw, kv.astype(bf16), preferred_element_type=f32)
        a, b = xh[:C], xh[C:]
        xs[slot][j, 0] = a
        xs[slot][j, 1] = b
        xs[slot][j, 2] = a + b
        kh = lax.dot_general(fw, sb[c, :, aligned(j, C)], (((1,), (1,)), ((), ())),
                             preferred_element_type=f32)
        kc, kd = kh[:C], kh[C:]
        if j == 0:
            kc = kc + ssd[:, lo:hi]
            cc, dd = kc, kd
        else:
            cc = kc - sigma * kprev[1]
            dd = kd + sigma * kprev[0]
        kprev[0] = kc
        kprev[1] = kd
        ks[slot][j, 0] = cc
        ks[slot][j, 1] = dd - cc
        ks[slot][j, 2] = cc + dd

    def stage_b(c, ft):
        slot = c % 2
        rows = aligned(ft, 8)
        IB = 4
        for i0 in range(0, NC, IB):
            acc = [[None] * 3 for _ in range(IB)]
            kreg = {}
            for j in range(i0 + IB):
                xa, xb, xab = (xs[slot][j, 2, rows, :], xs[slot][j, 0, rows, :], xs[slot][j, 1, rows, :])
                for ii in range(IB):
                    m = i0 + ii - j
                    if m < 0:
                        continue
                    if m not in kreg:
                        kreg[m] = tuple(ks[slot][m, p, rows, :] for p in range(3))
                    for p, xv in enumerate((xa, xb, xab)):
                        t = kreg[m][p] * xv
                        acc[ii][p] = t if acc[ii][p] is None else acc[ii][p] + t
                kreg.pop(i0 - j, None)
            for ii in range(IB):
                zs[slot][i0 + ii, rows, :] = acc[ii][0] - acc[ii][2]
                zs[slot][i0 + ii, pl.ds(C + ft * 8, 8), :] = acc[ii][0] + acc[ii][1]

    def stage_c(c, i):
        slot = c % 2
        y = jnp.dot(inv_ref[...], zs[slot][i].astype(bf16), preferred_element_type=f32)
        ys[c][aligned(i, C), :] = y

    for c in range(-1, NT + 1):
        if 0 <= c + 1 < NT:
            if True:
                for cp in slab(c + 1):
                    cp.wait()
            for cp in {0: (cp_wm,), 1: (cp_q, cp_w1, cp_w2)}.get(c, ()):
                cp.start()

        if c == NT - 1:
            cp_wm.wait()
            cv = c_ref[...].astype(f32)
            sc = jnp.broadcast_to((cv * jax.nn.sigmoid(cv)).astype(bf16), (8, D))

        def body(t, _, c=c):
            if c == NT - 1 and t < 15:
                cols = aligned(t, 256)
                modb[:, cols] = jnp.dot(sc, wmb[:, cols], preferred_element_type=f32)
            if 0 <= c + 1 < NT:
                stage_a(c + 1, t)
            if 0 <= c < NT:
                stage_b(c, t)
            if 0 <= c - 1 < NT:
                stage_c(c - 1, t)
            return 0
        if True:
            for t in range(NC):
                body(t, 0)

    if True:
        mod = modb[0:1, :]
        sa, ca, ga, sbb, cb, gb = (mod[:, n * D:(n + 1) * D] for n in range(6))
        b1 = b1_ref[...].reshape(1, F).astype(f32)
        b2 = b2_ref[...].reshape(1, D).astype(f32)
        cp_q.wait()
        cp_w1.wait()
        cp_w2.wait()

    def out_copy(r, slot):
        return pltpu.make_async_copy(ob.at[slot], o_h.at[0, aligned(r, TM), :], sem_o.at[slot])

    x1b, h2b = (x1a, x1c), (h2a, h2c)

    def prep(r, slot):
        rows = aligned(r, TM)
        x0 = qb[rows, :].astype(f32)
        y = jnp.concatenate([ys[c][rows, :] for c in range(NT)], axis=1)
        x1 = x0 + ga * ((_ln(x0) * (1.0 + ca) + sa) * y)
        x1b[slot][...] = x1
        hn = (_ln(x1) * (1.0 + cb) + sbb).astype(bf16)
        h2b[slot][...] = hn
        return hn

    prep(0, 0)

    def ffn(r, slot, oslot):
        h2 = h2b[slot][...]
        x1 = x1b[slot][...]
        hn = prep(jnp.minimum(r + 1, S // TM - 1), 1 - slot)
        o = b2
        for lo, hi in zip(FCUTS[:-1], FCUTS[1:]):
            h = lax.dot_general(h2, w1b[lo:hi, :], (((1,), (1,)), ((), ())), preferred_element_type=f32) + b1[:, lo:hi]
            g = jax.nn.gelu(h, approximate=True).astype(bf16)
            if lo == 0:
                h2 = jnp.where(r < 0, hn, h2)
            o = o + jnp.dot(g, w2b[lo:hi, :], preferred_element_type=f32)

        ob[oslot] = (x1 + gb * o).astype(bf16)

    def pair(p, _):
        o0 = 2 * (p % 2)

        @pl.when(p >= 2)
        def _():
            out_copy(2 * p - 4, o0).wait()
            out_copy(2 * p - 3, o0 + 1).wait()
        ffn(2 * p, 0, o0)
        ffn(2 * p + 1, 1, o0 + 1)
        out_copy(2 * p, o0).start()
        out_copy(2 * p + 1, o0 + 1).start()
        return 0
    if True:
        lax.fori_loop(0, S // TM // 2, pair, 0)
    for r in range(S // TM - 4, S // TM):
        out_copy(r, r % 4).wait()


@jax.jit
def pallas_adaLN_cond__ssm_conv_h3__dense_activation_gelu__prompt_kernel(
    A_q, A_k, A_v, A_shift_k, A_ssm_k, A_ssm_D, B_x, B_w1, B_b1, B_w2, B_b2, c, w_mod,
):
    del B_x
    fwd, inv = _dft_consts()
    hbm = pl.BlockSpec(memory_space=pltpu.HBM)
    vm = pl.BlockSpec(memory_space=pltpu.VMEM)
    return pl.pallas_call(
        _kernel,
        in_specs=[hbm, hbm, hbm, vm, hbm, vm, hbm, vm, hbm, vm, vm, hbm, vm, vm],
        out_specs=hbm,
        out_shape=jax.ShapeDtypeStruct((1, S, D), bf16),
        scratch_shapes=[
            pltpu.VMEM((S, D), bf16),
            pltpu.VMEM((NT, S + HALO, 128), bf16),
            pltpu.VMEM((NT, S, 128), bf16),
            pltpu.VMEM((NT, 128, S), bf16),
            pltpu.VMEM((F, D), bf16),
            pltpu.VMEM((F, D), bf16),
            pltpu.VMEM((D, 6 * D), bf16),
            pltpu.VMEM((2, C, 128), f32),
            pltpu.VMEM((8, 6 * D), f32),
            pltpu.VMEM((4, TM, D), bf16),
            pltpu.VMEM((TM, D), f32),
            pltpu.VMEM((TM, D), f32),
            pltpu.VMEM((TM, D), bf16),
            pltpu.VMEM((TM, D), bf16),
            pltpu.SemaphoreType.DMA((3, NT)),
            pltpu.SemaphoreType.DMA((4,)),
            pltpu.SemaphoreType.DMA((4,)),
        ] + [pltpu.VMEM((S, 128), f32)] * NT
          + [pltpu.VMEM((NC, 3, C, 128), f32)] * 4
          + [pltpu.VMEM((NC, 2 * C, 128), f32)] * 2
          + [pltpu.VMEM((8 + S, 128), f32)] * 2,
        compiler_params=pltpu.CompilerParams(vmem_limit_bytes=100 * 1024 * 1024),
    )(A_q, A_k, A_v, A_shift_k.T, A_ssm_k, A_ssm_D, B_w1.T, B_b1,
      B_w2, B_b2, c, w_mod, jnp.asarray(fwd, bf16), jnp.asarray(inv, bf16))
```

```python
import numpy as np
import jax
import jax.numpy as jnp
from jax import lax
import jax.experimental.pallas as pl
import jax.experimental.pallas.tpu as pltpu

S, D, F = 2048, 640, 1728
C = 128
NC = S // C
NT = D // 128
HALO = 16
FCUTS = (0,1024,F)
G = 2
TM = 256
f32, bf16 = jnp.float32, jnp.bfloat16


def _dft_consts():
    f = np.arange(C, dtype=np.float64)[:, None] + 0.5
    t = np.arange(C, dtype=np.float64)[None, :]
    th = 2.0 * np.pi * f * t / (2 * C)
    fwd = np.concatenate([np.cos(th), -np.sin(th)], axis=0)
    inv = np.concatenate([np.cos(th).T, -np.sin(th).T], axis=1) / C
    return fwd.astype(np.float32), inv.astype(np.float32)


def _ln(x):
    m = jnp.mean(x, axis=-1, keepdims=True)
    xc = x - m
    v = jnp.mean(xc * xc, axis=-1, keepdims=True)
    return xc * lax.rsqrt(v + 1e-5)


def _kernel(q_h, k_h, v_h, shk_ref, ssm_h, ssd_ref, w1_h, b1_ref, w2_h, b2_ref, c_ref, wm_h,
            fwd_ref, inv_ref, o_h,
            qb, kb, vb, sb, w1b, w2b, wmb, kprev, modb, ob, x1a, x1c, h2a, h2c, sem_in, sem_w, sem_o, *rest):
    ys = rest[:NT]
    kfs = rest[NT + 6:NT + 8]
    xs, ks, zs = (rest[NT + 2 * n:NT + 2 * n + 2] for n in range(3))
    def slab(c):
        cols = pl.ds(c * 128, 128)
        return (pltpu.make_async_copy(k_h.at[0, :, cols], kb.at[c, pl.ds(HALO, S)], sem_in.at[0, c]),
                pltpu.make_async_copy(v_h.at[0, :, cols], vb.at[c], sem_in.at[1, c]),
                pltpu.make_async_copy(ssm_h.at[cols, :], sb.at[c], sem_in.at[2, c]))
    for c in range(NT):
        for cp in slab(c):
            cp.start()
    cp_wm = pltpu.make_async_copy(wm_h, wmb, sem_w.at[0])
    cp_q = pltpu.make_async_copy(q_h.at[0], qb, sem_w.at[1])
    cp_w1 = pltpu.make_async_copy(w1_h, w1b, sem_w.at[2])
    cp_w2 = pltpu.make_async_copy(w2_h, w2b, sem_w.at[3])

    for c in range(NT):
        kb[c, pl.ds(0, HALO), :] = jnp.zeros((HALO, 128), bf16)


    taps = shk_ref[...].astype(f32)
    ssd = ssd_ref[...].reshape(1, D).astype(f32)
    sigma = (1 - 2 * (lax.broadcasted_iota(jnp.int32, (C, 128), 0) & 1)).astype(f32)

    def aligned(i, n):
        return pl.ds(i * n if isinstance(i, int) else pl.multiple_of(i * n, n), n)

    def stage_a(c, j):
        slot = c % 2
        lo, hi = c * 128, (c + 1) * 128
        w = kb[c, pl.ds(HALO + j * C, C), :].astype(f32)
        kf = kfs[slot]
        if j == 0:
            kf[pl.ds(0, 8), :] = jnp.zeros((8, 128), f32)
        kf[pl.ds(8 + j * C, C), :] = w
        ksh = w * taps[0:1, lo:hi]
        for s in range(1, 4):
            ksh = ksh + kf[pl.ds(8 + j * C - s, C), :] * taps[s:s + 1, lo:hi]
        kv = ksh * vb[c, aligned(j, C), :].astype(f32)
        fw = fwd_ref[...]
        xh = jnp.dot(fw, kv.astype(bf16), preferred_element_type=f32)
        a, b = xh[:C], xh[C:]
        xs[slot][j, 0] = a
        xs[slot][j, 1] = b
        xs[slot][j, 2] = a + b
        kh = lax.dot_general(fw, sb[c, :, aligned(j, C)], (((1,), (1,)), ((), ())),
                             preferred_element_type=f32)
        kc, kd = kh[:C], kh[C:]
        if j == 0:
            kc = kc + ssd[:, lo:hi]
            cc, dd = kc, kd
        else:
            cc = kc - sigma * kprev[1]
            dd = kd + sigma * kprev[0]
        kprev[0] = kc
        kprev[1] = kd
        ks[slot][j, 0] = cc
        ks[slot][j, 1] = dd - cc
        ks[slot][j, 2] = cc + dd

    def stage_b(c, ft):
        slot = c % 2
        rows = aligned(ft, 8)
        IB = 4
        for i0 in range(0, NC, IB):
            acc = [[None] * 3 for _ in range(IB)]
            kreg = {}
            for j in range(i0 + IB):
                xa, xb, xab = (xs[slot][j, 2, rows, :], xs[slot][j, 0, rows, :], xs[slot][j, 1, rows, :])
                for ii in range(IB):
                    m = i0 + ii - j
                    if m < 0:
                        continue
                    if m not in kreg:
                        kreg[m] = tuple(ks[slot][m, p, rows, :] for p in range(3))
                    for p, xv in enumerate((xa, xb, xab)):
                        t = kreg[m][p] * xv
                        acc[ii][p] = t if acc[ii][p] is None else acc[ii][p] + t
                kreg.pop(i0 - j, None)
            for ii in range(IB):
                zs[slot][i0 + ii, rows, :] = acc[ii][0] - acc[ii][2]
                zs[slot][i0 + ii, pl.ds(C + ft * 8, 8), :] = acc[ii][0] + acc[ii][1]

    def stage_c(c, i):
        slot = c % 2
        y = jnp.dot(inv_ref[...], zs[slot][i].astype(bf16), preferred_element_type=f32)
        ys[c][aligned(i, C), :] = y

    for c in range(-1, NT + 1):
        if 0 <= c + 1 < NT:
            if True:
                for cp in slab(c + 1):
                    cp.wait()
            for cp in {0: (cp_wm,), 1: (cp_q, cp_w1, cp_w2)}.get(c, ()):
                cp.start()

        if c == NT - 1:
            cp_wm.wait()
            cv = c_ref[...].astype(f32)
            sc = jnp.broadcast_to((cv * jax.nn.sigmoid(cv)).astype(bf16), (8, D))

        def body(t, _, c=c):
            if c == NT - 1 and t < 15:
                cols = aligned(t, 256)
                modb[:, cols] = jnp.dot(sc, wmb[:, cols], preferred_element_type=f32)
            if 0 <= c + 1 < NT:
                stage_a(c + 1, t)
            if 0 <= c < NT:
                stage_b(c, t)
            if 0 <= c - 1 < NT:
                stage_c(c - 1, t)
            return 0
        if True:
            for t in range(NC):
                body(t, 0)

    if True:
        mod = modb[0:1, :]
        sa, ca, ga, sbb, cb, gb = (mod[:, n * D:(n + 1) * D] for n in range(6))
        b1 = b1_ref[...].reshape(1, F).astype(f32)
        b2 = b2_ref[...].reshape(1, D).astype(f32)
        cp_q.wait()
        cp_w1.wait()
        cp_w2.wait()

    def out_copy(r, slot):
        return pltpu.make_async_copy(ob.at[slot], o_h.at[0, aligned(r, TM), :], sem_o.at[slot])

    x1b, h2b = (x1a, x1c), (h2a, h2c)

    def prep(r, slot):
        rows = aligned(r, TM)
        x0 = qb[rows, :].astype(f32)
        y = jnp.concatenate([ys[c][rows, :] for c in range(NT)], axis=1)
        x1 = x0 + ga * ((_ln(x0) * (1.0 + ca) + sa) * y)
        x1b[slot][...] = x1
        hn = (_ln(x1) * (1.0 + cb) + sbb).astype(bf16)
        h2b[slot][...] = hn
        return hn

    prep(0, 0)

    def ffn(r, slot, oslot):
        h2 = h2b[slot][...]
        x1 = x1b[slot][...]
        hn = prep(jnp.minimum(r + 1, S // TM - 1), 1 - slot)
        o = b2
        for lo, hi in zip(FCUTS[:-1], FCUTS[1:]):
            h = lax.dot_general(h2, w1b[lo:hi, :], (((1,), (1,)), ((), ())), preferred_element_type=f32) + b1[:, lo:hi]
            g = jax.nn.gelu(h, approximate=True).astype(bf16)
            if lo == 0:
                h2 = jnp.where(r < 0, hn, h2)
            o = o + jnp.dot(g, w2b[lo:hi, :], preferred_element_type=f32)

        ob[oslot] = (x1 + gb * o).astype(bf16)

    def group(p, _):
        for n in range(G):
            ffn(G * p + n, n % 2, G * p + n)
        for n in range(G):
            out_copy(G * p + n, G * p + n).start()
        return 0
    lax.fori_loop(0, S // TM // G, group, 0)
    for r in range(S // TM):
        out_copy(r, r).wait()


@jax.jit
def pallas_adaLN_cond__ssm_conv_h3__dense_activation_gelu__prompt_kernel(
    A_q, A_k, A_v, A_shift_k, A_ssm_k, A_ssm_D, B_x, B_w1, B_b1, B_w2, B_b2, c, w_mod,
):
    del B_x
    fwd, inv = _dft_consts()
    hbm = pl.BlockSpec(memory_space=pltpu.HBM)
    vm = pl.BlockSpec(memory_space=pltpu.VMEM)
    return pl.pallas_call(
        _kernel,
        in_specs=[hbm, hbm, hbm, vm, hbm, vm, hbm, vm, hbm, vm, vm, hbm, vm, vm],
        out_specs=hbm,
        out_shape=jax.ShapeDtypeStruct((1, S, D), bf16),
        scratch_shapes=[
            pltpu.VMEM((S, D), bf16),
            pltpu.VMEM((NT, S + HALO, 128), bf16),
            pltpu.VMEM((NT, S, 128), bf16),
            pltpu.VMEM((NT, 128, S), bf16),
            pltpu.VMEM((F, D), bf16),
            pltpu.VMEM((F, D), bf16),
            pltpu.VMEM((D, 6 * D), bf16),
            pltpu.VMEM((2, C, 128), f32),
            pltpu.VMEM((8, 6 * D), f32),
            pltpu.VMEM((S // TM, TM, D), bf16),
            pltpu.VMEM((TM, D), f32),
            pltpu.VMEM((TM, D), f32),
            pltpu.VMEM((TM, D), bf16),
            pltpu.VMEM((TM, D), bf16),
            pltpu.SemaphoreType.DMA((3, NT)),
            pltpu.SemaphoreType.DMA((4,)),
            pltpu.SemaphoreType.DMA((S // TM,)),
        ] + [pltpu.VMEM((S, 128), f32)] * NT
          + [pltpu.VMEM((NC, 3, C, 128), f32)] * 4
          + [pltpu.VMEM((NC, 2 * C, 128), f32)] * 2
          + [pltpu.VMEM((8 + S, 128), f32)] * 2,
        compiler_params=pltpu.CompilerParams(vmem_limit_bytes=100 * 1024 * 1024),
    )(A_q, A_k, A_v, A_shift_k.T, A_ssm_k, A_ssm_D, B_w1.T, B_b1,
      B_w2, B_b2, c, w_mod, jnp.asarray(fwd, bf16), jnp.asarray(inv, bf16))
```
